```python
import os as _os
_os.environ.setdefault('JAX_PLATFORMS', 'cpu')
import jax
import jax.numpy as jnp

def _softmax(x, axis=-1):
    return jax.nn.softmax(x, axis=axis)

def _gelu(x):
    return jax.nn.gelu(x, approximate=True)

def _silu(x):
    return jax.nn.silu(x)

def _sigmoid(x):
    return jax.nn.sigmoid(x)

def _layernorm(x, axis=-1, eps=1e-05):
    m = jnp.mean(x, axis=axis, keepdims=True)
    v = jnp.var(x, axis=axis, keepdims=True)
    return (x - m) / jnp.sqrt(v + eps)

def _scatter_add(tgt, idx, src, axis=0):
    return tgt.at[idx].add(src)

def _segment_sum(src, seg, n):
    return jax.ops.segment_sum(src, seg, n)

class _Rng:

    def __init__(self, key):
        self._k = key

    def _next(self):
        self._k, sub = jax.random.split(self._k)
        return sub

    def normal(self, shape):
        return jax.random.normal(self._next(), shape, dtype=jnp.bfloat16)

    def randint(self, lo, hi, shape):
        return jax.random.randint(self._next(), shape, lo, hi, dtype=jnp.int32)

    def uniform(self, shape, lo=0.0, hi=1.0):
        return jax.random.uniform(self._next(), shape, jnp.bfloat16, lo, hi)

    def permutation(self, n):
        return jax.random.permutation(self._next(), n)
kernel_name = 'parallel_sum__memory_aug_recurrent_mem_tr__dense_activation_silu__prompt'

def setup_inputs():
    _rng = _Rng(jax.random.key(int.from_bytes(__import__("os").urandom(4), "little")))
    _w = lambda a: (lambda t: t.astype(jnp.bfloat16) if jnp.issubdtype(t.dtype, jnp.floating) else t)(jnp.asarray(a))

    def _A_setup():
        B, S, Dm = (1, 2048, 448)
        H, Dh = (16, 256)
        M, seg = (8, 32)
        seg = min(seg, S)
        S = S // seg * seg
        return {'x': _w((lambda *s: _rng.normal(s) * 0.05)(B, S, Dm)), 'mem0': _w((lambda *s: _rng.normal(s) * 0.2)(B, M, Dm)), 'Wq': _w((lambda *s: _rng.normal(s) * 0.8)(Dm, H, Dh) * Dm ** (-0.5)), 'Wk': _w((lambda *s: _rng.normal(s) * 0.8)(Dm, H, Dh) * Dm ** (-0.5)), 'Wv': _w((lambda *s: _rng.normal(s) * 0.2)(Dm, H, Dh) * Dm ** (-0.5)), 'Wo': _w((lambda *s: _rng.normal(s) * 0.2)(H, Dh, Dm) * (H * Dh) ** (-0.5)), 'seg_len': seg}
    _A_in = _A_setup()

    def _B_setup():
        B, S, D, F = (1, 2048, 448, 1792)
        return {'x': _w((lambda *s: _rng.normal(s) * 0.05)(B, S, D)), 'w1': _w((lambda *s: _rng.normal(s) * 0.05)(D, F) * D ** (-0.5)), 'w2': _w((lambda *s: _rng.normal(s) * 0.05)(F, D) * F ** (-0.5))}
    _B_in = _B_setup()
    return {'A_x': _A_in['x'], 'A_mem0': _A_in['mem0'], 'A_Wq': _A_in['Wq'], 'A_Wk': _A_in['Wk'], 'A_Wv': _A_in['Wv'], 'A_Wo': _A_in['Wo'], 'A_seg_len': _A_in['seg_len'], 'B_x': _B_in['x'], 'B_w1': _B_in['w1'], 'B_w2': _B_in['w2']}

def reference(A_x, A_mem0, A_Wq, A_Wk, A_Wv, A_Wo, A_seg_len, B_x, B_w1, B_w2):

    def _A_ref(x, mem0, Wq, Wk, Wv, Wo, seg_len):
        B, S, Dm = x.shape
        H, Dh = (Wq.shape[1], Wq.shape[2])
        M = mem0.shape[1]
        scale = Dh ** (-0.5)
        n_seg = S // seg_len
        L = M + seg_len
        idx = jnp.arange(L)
        mask = (idx[:, None] < M) | (idx[:, None] >= idx[None, :])
        mem = mem0
        outs = []
        for s in range(n_seg):
            xs = x[:, s * seg_len:(s + 1) * seg_len, :].copy()
            h = jnp.concatenate([mem, xs], axis=1)
            q = jnp.einsum('btd,dhe->bhte', h, Wq)
            k = jnp.einsum('btd,dhe->bhte', h, Wk)
            v = jnp.einsum('btd,dhe->bhte', h, Wv)
            scores = jnp.einsum('bhqe,bhke->bhqk', q, k) * scale
            scores = jnp.where(mask[None, None], scores, -1000000000.0)
            p = _softmax(scores, axis=-1)
            o = jnp.einsum('bhqk,bhke->bhqe', p, v)
            o = jnp.einsum('bhte,hed->btd', o, Wo)
            mem = o[:, :M, :].copy()
            outs.append(o[:, M:, :])
        return jnp.concatenate(outs, axis=1)

    def _B_ref(x, w1, w2):
        h = jnp.einsum('bsd,df->bsf', x, w1)
        h = _silu(h)
        out = jnp.einsum('bsf,fd->bsd', h, w2)
        return out
    x = A_x
    xn = _layernorm(x, axis=-1)
    return x + _A_ref(xn, A_mem0, A_Wq, A_Wk, A_Wv, A_Wo, A_seg_len) + _B_ref(xn, B_w1, B_w2)
```

```python
import functools

import jax
import jax.numpy as jnp
import numpy as np
from jax.experimental import pallas as pl
from jax.experimental.pallas import tpu as pltpu

_F32 = jnp.float32
_BF16 = jnp.bfloat16
_U32 = jnp.uint32


def _dot(a, b):
    return jax.lax.dot_general(a, b, (((1,), (0,)), ((), ())), preferred_element_type=_F32)


def _dot_nt(a, b):
    return jax.lax.dot_general(a, b, (((1,), (1,)), ((), ())), preferred_element_type=_F32)


def _make_kernel(S, D, DP, H, E, M, SEG, F):
    n_seg = S // SEG
    L = M + SEG
    FB = 256
    OC = 512
    scale = float(E) ** -0.5
    NST = int(n_seg)

    def kernel(xt_hbm, mem_hbm, wq_hbm, wk_hbm, wv_hbm, wot_hbm, w1_hbm, w2t_hbm, outt_hbm,
               xt, mem0_s, raw_q, raw_k, raw_v, raw_o, raw_1, raw_2,
               xn, base, wqkv, wo, w1, w2t, o_s, out_s, outt_s, sems, osem):
        cp_x = pltpu.make_async_copy(xt_hbm, xt.at[pl.ds(0, D)], sems.at[0])
        cp_1 = pltpu.make_async_copy(w1_hbm, raw_1, sems.at[1])
        cp_2 = pltpu.make_async_copy(w2t_hbm, raw_2, sems.at[2])
        cp_m = pltpu.make_async_copy(mem_hbm, mem0_s, sems.at[3])
        cp_qkv = []
        for i, (src, dst) in enumerate(((wq_hbm, raw_q), (wk_hbm, raw_k), (wv_hbm, raw_v))):
            for ec in range(E // 128):
                cp_qkv.append(pltpu.make_async_copy(
                    src.at[:, pl.ds(ec * 128, 128)], dst.at[ec], sems.at[4 + 2 * i + ec]))
        cp_o = pltpu.make_async_copy(wot_hbm, raw_o, sems.at[10])
        for c in [cp_x, cp_1, cp_2, cp_m] + cp_qkv + [cp_o]:
            c.start()

        def pack_rows_padded(raw_ref, dst_ref, N):
            CH = 64
            def body(i, _):
                r = pl.multiple_of(i * CH, CH)
                dst_ref[pl.ds(pl.multiple_of(i * (CH // 2), CH // 2), CH // 2), :] = pltpu.bitcast(
                    raw_ref[pl.ds(r, CH), :], _U32)
                return _
            jax.lax.fori_loop(0, D // CH, body, 0)
            dst_ref[pl.ds(D // 2, (DP - D) // 2), :] = jnp.zeros(((DP - D) // 2, N), _U32)

        xt[pl.ds(D, DP - D), :] = jnp.zeros((DP - D, S), _BF16)
        cp_x.wait()
        lane = jax.lax.broadcasted_iota(jnp.int32, (FB, DP), 1)

        def ln_body(i, _):
            r = pl.multiple_of(i * FB, FB)
            xf = xt[:, pl.ds(r, FB)].T.astype(_F32)
            mu = jnp.sum(xf, axis=1, keepdims=True) * (1.0 / D)
            c = jnp.where(lane < D, xf - mu, 0.0)
            var = jnp.sum(c * c, axis=1, keepdims=True) * (1.0 / D)
            xn[pl.ds(r, FB), :] = c * jax.lax.rsqrt(var + 1e-5)
            base[pl.ds(r, FB), :] = xf
            return _
        jax.lax.fori_loop(0, S // FB, ln_body, 0)

        cp_1.wait()
        pack_rows_padded(raw_1, w1, F)
        cp_2.wait()
        pack_rows_padded(raw_2, w2t, F)

        def ffn_body(i, _):
            r = pl.multiple_of(i * FB, FB)
            hid = _dot(xn[pl.ds(r, FB), :], pltpu.bitcast(w1[...], _BF16))
            act = hid * jax.nn.sigmoid(hid)
            y = _dot_nt(act, pltpu.bitcast(w2t[...], _BF16))
            base[pl.ds(r, FB), :] += y
            return _
        jax.lax.fori_loop(0, S // FB, ffn_body, 0)

        for c in cp_qkv:
            c.wait()
        wqkv[:, pl.ds(D // 2, (DP - D) // 2), :] = jnp.zeros((H, (DP - D) // 2, 3 * E), _U32)
        for wi, raw in enumerate((raw_q, raw_k, raw_v)):
            ru = raw.bitcast(_U32)
            for ec in range(E // 128):
                for p in range(H // 2):
                    a = ru[ec, pl.ds(p, D, stride=H // 2), :]
                    lo = pltpu.bitcast(a << 16, _F32).astype(_BF16)
                    hi = pltpu.bitcast(a & _U32(0xFFFF0000), _F32).astype(_BF16)
                    col = pl.ds(wi * E + ec * 128, 128)
                    wqkv[2 * p, pl.ds(0, D // 2), col] = pltpu.bitcast(lo, _U32)
                    wqkv[2 * p + 1, pl.ds(0, D // 2), col] = pltpu.bitcast(hi, _U32)
        cp_o.wait()
        for h in range(H):
            wt = jnp.concatenate([raw_o[pl.ds(h * D, D), :], jnp.zeros((DP - D, E), _BF16)], axis=0)
            wo[pl.ds(h * (E // 2), E // 2), :] = pltpu.bitcast(wt.T, _U32)
        cp_m.wait()

        row = jax.lax.broadcasted_iota(jnp.int32, (L, L), 0)
        col = jax.lax.broadcasted_iota(jnp.int32, (L, L), 1)
        mask = (row < M) | (row >= col)

        def flush(c):
            r = pl.multiple_of(c * OC, OC)
            outt_s[:, pl.ds(r, OC)] = out_s[pl.ds(r, OC), :].T
            pltpu.make_async_copy(outt_s.at[pl.ds(0, D), pl.ds(r, OC)],
                                  outt_hbm.at[:, pl.ds(r, OC)], osem).start()

        def step(s, mem):
            r = pl.multiple_of(s * SEG, SEG)
            hl = jnp.concatenate([mem, xn[pl.ds(r, SEG), :]], axis=0)
            VAR = "full"
            D1 = int("2"); D2 = int("4")
            qkv = {}; pp = {}
            def stage_q(h):
                qkv[h] = _dot(hl, pltpu.bitcast(wqkv[h], _BF16))
            def stage_s(h):
                y = qkv[h]
                q = y[:, :E]
                k = y[:, E:2 * E].astype(_BF16)
                sc = jnp.where(mask, _dot_nt(q, k) * scale, -1e9)
                mx = jnp.max(sc, axis=1, keepdims=True)
                e = jnp.exp(sc - mx)
                pp[h] = e / jnp.sum(e, axis=1, keepdims=True)
            def stage_p(h):
                v = qkv[h][:, 2 * E:].astype(_BF16)
                o_s[:, h * E:(h + 1) * E] = _dot(pp[h], v)
            for t in range(H + D2):
                if t < H: stage_q(t)
                if 0 <= t - D1 < H: stage_s(t - D1)
                if 0 <= t - D2 < H: stage_p(t - D2)
            a = _dot(o_s[...], pltpu.bitcast(wo[...], _BF16))
            out_s[pl.ds(r, SEG), :] = (base[pl.ds(r, SEG), :] + a[M:, :]).astype(_BF16)

            if NST == n_seg:
                @pl.when(jnp.logical_and((s + 1) % (OC // SEG) == 0, s + 1 < n_seg))
                def _():
                    flush((s + 1) // (OC // SEG) - 1)
            return a[:M, :]

        m0 = jnp.concatenate([mem0_s[...].astype(_F32), jnp.zeros((M, DP - D), _F32)], axis=1)
        jax.lax.fori_loop(0, NST, step, m0)
        flush(S // OC - 1)
        if NST == n_seg:
            pltpu.make_async_copy(outt_s.at[pl.ds(0, D)], outt_hbm, osem).wait()
        else:
            pltpu.make_async_copy(outt_s.at[pl.ds(0, D), pl.ds(0, OC)], outt_hbm.at[:, pl.ds(0, OC)], osem).wait()

    return kernel


@functools.partial(jax.jit, static_argnames=("A_seg_len",))
def pallas_parallel_sum__memory_aug_recurrent_mem_tr__dense_activation_silu__prompt_kernel(
    A_x, A_mem0, A_Wq, A_Wk, A_Wv, A_Wo, A_seg_len, B_x, B_w1, B_w2,
):
    del B_x
    B, S, D = A_x.shape
    M = A_mem0.shape[1]
    _, H, E = A_Wq.shape
    F = B_w1.shape[1]
    SEG = int(A_seg_len)
    DP = -(-D // 128) * 128
    assert B == 1 and S % SEG == 0 and S % 512 == 0
    L = M + SEG
    kernel = _make_kernel(S, D, DP, H, E, M, SEG, F)
    hbm = pl.BlockSpec(memory_space=pltpu.HBM)
    out_t = pl.pallas_call(
        kernel,
        out_shape=pltpu.HBM((D, S), A_x.dtype),
        in_specs=[hbm] * 8,
        out_specs=hbm,
        scratch_shapes=[
            pltpu.VMEM((DP, S), _BF16),
            pltpu.VMEM((M, D), _BF16),
            pltpu.VMEM((E // 128, D * H, 128), _BF16),
            pltpu.VMEM((E // 128, D * H, 128), _BF16),
            pltpu.VMEM((E // 128, D * H, 128), _BF16),
            pltpu.VMEM((H * D, E), _BF16),
            pltpu.VMEM((D, F), _BF16),
            pltpu.VMEM((D, F), _BF16),
            pltpu.VMEM((S, DP), _F32),
            pltpu.VMEM((S, DP), _F32),
            pltpu.VMEM((H, DP // 2, 3 * E), _U32),
            pltpu.VMEM((H * E // 2, DP), _U32),
            pltpu.VMEM((DP // 2, F), _U32),
            pltpu.VMEM((DP // 2, F), _U32),
            pltpu.VMEM((L, H * E), _F32),
            pltpu.VMEM((S, DP), _BF16),
            pltpu.VMEM((DP, S), _BF16),
            pltpu.SemaphoreType.DMA((11,)),
            pltpu.SemaphoreType.DMA(()),
        ],
        compiler_params=pltpu.CompilerParams(vmem_limit_bytes=110 * 1024 * 1024),
    )(
        A_x.reshape(S, D).T, A_mem0.reshape(M, D),
        A_Wq.reshape(D * H, E), A_Wk.reshape(D * H, E), A_Wv.reshape(D * H, E),
        A_Wo.transpose(0, 2, 1).reshape(H * D, E), B_w1, B_w2.T,
    )
    return out_t.T.reshape(B, S, D)
```

```python
import functools

import jax
import jax.numpy as jnp
import numpy as np
from jax.experimental import pallas as pl
from jax.experimental.pallas import tpu as pltpu

_F32 = jnp.float32
_BF16 = jnp.bfloat16
_U32 = jnp.uint32


def _dot(a, b):
    return jax.lax.dot_general(a, b, (((1,), (0,)), ((), ())), preferred_element_type=_F32)


def _dot_nt(a, b):
    return jax.lax.dot_general(a, b, (((1,), (1,)), ((), ())), preferred_element_type=_F32)


def _aligned(i, n):
    return i if isinstance(i, int) else pl.multiple_of(i, n)


def _make_kernel(S, D, DP, H, E, M, SEG, F):
    n_seg = S // SEG
    HP = DP // 2 + 8
    hpos = lambda h: (h % 2) * (H // 2) + h // 2
    L = M + SEG
    FB = 256
    OC = 512
    CW = 256
    NB = S // FB
    NBB = 3
    scale = float(E) ** -0.5
    NST = int(n_seg)
    D1, D2, G = int("2"), int("5"), int("2")

    def kernel(xt_hbm, mem_hbm, wq_hbm, wk_hbm, wv_hbm, wot_hbm, w1_hbm, w2t_hbm, outt_hbm,
               xt, mem0_s, raw_w, raw_o, raw_1, w2t,
               xn, baset, wqkv, wo, w1, o_s, out_s, outt_s, act_s, zero_s, sems, osem):
        cp_x0 = pltpu.make_async_copy(xt_hbm.at[:, pl.ds(0, FB)], xt.at[pl.ds(0, D), pl.ds(0, FB)], sems.at[0])
        cp_x1 = pltpu.make_async_copy(xt_hbm.at[:, pl.ds(FB, FB)], xt.at[pl.ds(0, D), pl.ds(FB, FB)], sems.at[11])
        cp_x2 = pltpu.make_async_copy(xt_hbm.at[:, pl.ds(2 * FB, S - 2 * FB)],
                                      xt.at[pl.ds(0, D), pl.ds(2 * FB, S - 2 * FB)], sems.at[12])
        cp_1 = pltpu.make_async_copy(w1_hbm, raw_1, sems.at[1])
        cp_2 = pltpu.make_async_copy(w2t_hbm, w2t, sems.at[2])
        cp_m = pltpu.make_async_copy(mem_hbm, mem0_s, sems.at[3])
        cp_att = []
        for i, src in enumerate((wq_hbm, wk_hbm, wv_hbm)):
            for ec in range(E // 128):
                cp_att.append(pltpu.make_async_copy(
                    src.at[:, pl.ds(ec * 128, 128)], raw_w.at[i * (E // 128) + ec], sems.at[4 + 2 * i + ec]))
        cp_att.append(pltpu.make_async_copy(wot_hbm, raw_o, sems.at[10]))
        DMAO = "1"
        for c in [cp_x0, cp_1, cp_2, cp_x1, cp_x2, cp_m] + (cp_att if DMAO == "0" else []):
            c.start()

        xt[pl.ds(D, DP - D), :] = jnp.zeros((DP - D, S), _BF16)
        for h in range(H):
            wqkv[:, pl.ds(h * HP + D // 2, (DP - D) // 2), :] = jnp.zeros((3 * E // 128, (DP - D) // 2, 128), _U32)
        w1[pl.ds(D // 2, (DP - D) // 2), :] = jnp.zeros(((DP - D) // 2, F), _U32)
        zero_s[...] = jnp.zeros((8, 128), _U32)
        lane = jax.lax.broadcasted_iota(jnp.int32, (FB, DP), 1)

        def layer_norm(i):
            r = _aligned(i * FB, FB)
            xf = xt[:, pl.ds(r, FB)].T.astype(_F32)
            mu = jnp.sum(xf, axis=1, keepdims=True) * (1.0 / D)
            c = jnp.where(lane < D, xf - mu, 0.0)
            var = jnp.sum(c * c, axis=1, keepdims=True) * (1.0 / D)
            xn[pl.ds(r, FB), :] = c * jax.lax.rsqrt(var + 1e-5)

        def xpose8(A):
            sub = jax.lax.broadcasted_iota(jnp.int32, A[0].shape, 0)
            A = list(A)
            for k in (4, 2, 1):
                m = (sub & k) != 0
                B = list(A)
                for i in range(8):
                    if i & k == 0:
                        B[i] = jnp.where(m, pltpu.roll(A[i + k], k, 0), A[i])
                        B[i + k] = jnp.where(m, A[i + k], pltpu.roll(A[i], 8 - k, 0))
                A = B
            return A

        def retile_qkv(j, zero):
            ru = raw_w.bitcast(_U32)
            dep = zero
            RT = "st"
            for ec in range(E // 128):
                jj = j * (E // 128) + ec
                for g in range(D // 16):
                    if RT == "st":
                        for i in range(8):
                            ev = ru[jj, pl.ds((16 * g + 2 * i) * 8, 8), :] | dep
                            od = ru[jj, pl.ds((16 * g + 2 * i + 1) * 8, 8), :] | dep
                            lo = (ev & _U32(0xFFFF)) | (od << 16)
                            last = (ev >> 16) | (od & _U32(0xFFFF0000))
                            wqkv[jj, pl.ds(8 * g + i, H // 2, stride=HP), :] = lo
                            wqkv[jj, pl.ds((H // 2) * HP + 8 * g + i, H // 2, stride=HP), :] = last
                    else:
                        ev = xpose8([ru[jj, pl.ds((16 * g + 2 * i) * 8, 8), :] | dep for i in range(8)])
                        od = xpose8([ru[jj, pl.ds((16 * g + 2 * i + 1) * 8, 8), :] | dep for i in range(8)])
                        for p in range(H // 2):
                            wqkv[jj, pl.ds(hpos(2 * p) * HP + g * 8, 8), :] = (ev[p] & _U32(0xFFFF)) | (od[p] << 16)
                            last = (ev[p] >> 16) | (od[p] & _U32(0xFFFF0000))
                            wqkv[jj, pl.ds(hpos(2 * p + 1) * HP + g * 8, 8), :] = last
                    if "1" == "1":
                        dep = pltpu.roll(last & zero, 1, 1)

        def retile_o(h):
            wt = jnp.concatenate([raw_o[pl.ds(_aligned(h * D, 64), D), :], jnp.zeros((DP - D, E), _BF16)], axis=0)
            wo[pl.ds(_aligned(h * (E // 2), E // 2), E // 2), :] = pltpu.bitcast(wt.T, _U32)

        def ffn_up(i, after_load=None):
            xb = xn[pl.ds(_aligned(i * FB, FB), FB), :]
            if after_load is not None:
                after_load()
            for c in range(F // CW):
                half = _dot(xb, pltpu.bitcast(w1[:, pl.ds(c * CW, CW)], _BF16)) * 0.5
                act_s[:, pl.ds(c * CW, CW)] = (half * jnp.tanh(half) + half).astype(_BF16)

        def ffn_down(i, between=None):
            cols = pl.ds(_aligned(i * FB, FB), FB)
            NC = int("2")
            w = D // NC
            for n in range(NC):
                rows = pl.ds(n * w, w)
                yt = _dot_nt(w2t[rows, :], act_s[...])
                baset[rows, cols] = yt + xt[rows, cols].astype(_F32)
                if between is not None:
                    between(n)

        with jax.named_scope("first"):
            cp_x0.wait()
            layer_norm(0)
            cp_1.wait()

            def pack_w1(i, _):
                w1[pl.ds(pl.multiple_of(i * 32, 32), 32), :] = pltpu.bitcast(
                    raw_1[pl.ds(pl.multiple_of(i * 64, 64), 64), :], _U32)
                return _
            jax.lax.fori_loop(0, D // 64, pack_w1, 0)
            if DMAO == "1":
                for c in cp_att:
                    c.start()
            ffn_up(0)
        with jax.named_scope("wait_w2"):
            cp_2.wait()
            cp_x1.wait()
            if DMAO == "2":
                for c in cp_att:
                    c.start()
        with jax.named_scope("second"):
            ffn_down(0)
            layer_norm(1)

        cp_x2.wait()

        def ffn_a(i, _):
            LP = "2"
            if LP == "0":
                ffn_up(i, lambda: layer_norm(i + 1))
                ffn_down(i)
            elif LP == "1":
                ffn_up(i)
                layer_norm(i + 1)
                ffn_down(i)
            else:
                ffn_up(i)
                ffn_down(i)
                layer_norm(i + 1)
            return _
        with jax.named_scope("loopA"):
            jax.lax.fori_loop(1, NB - NBB, ffn_a, 0)

        with jax.named_scope("wait_att"):
            for c in cp_att:
                c.wait()
            cp_m.wait()

        def ffn_b(j, _):
            retile_qkv(j, zero_s[...])
            LP = "2"
            lnb = lambda: layer_norm(jnp.minimum(j + (NB - NBB) + 1, NB - 1))
            ffn_up(j + NB - NBB, lnb if LP == "0" else None)
            if LP == "1":
                lnb()
            HH = -(-H // NBB)
            def between(n):
                NC = int("2")
                for hh in range(n * HH // NC, (n + 1) * HH // NC):
                    retile_o(jnp.minimum(j * HH + hh, H - 1))
            ffn_down(j + NB - NBB, between)
            if LP == "2":
                lnb()
            return _
        with jax.named_scope("loopB"):
            jax.lax.fori_loop(0, NBB, ffn_b, 0)

        row = jax.lax.broadcasted_iota(jnp.int32, (L, L), 0)
        col = jax.lax.broadcasted_iota(jnp.int32, (L, L), 1)
        mask = (row < M) | (row >= col)

        def flush(c):
            cols = pl.ds(_aligned(c * OC, OC), OC)
            at = out_s[cols, :].T
            outt_s[:, cols] = (baset[:, cols] + at[:D].astype(_F32)).astype(_BF16)
            pltpu.make_async_copy(outt_s.at[:, cols], outt_hbm.at[:, cols], osem).start()

        def step(s, mem):
            rows = pl.ds(pl.multiple_of(s * SEG, SEG), SEG)
            hl = jnp.concatenate([mem, xn[rows, :]], axis=0)
            qkv, pp, acc = {}, {}, []

            def stage_q(h):
                w = jnp.concatenate([wqkv[ct, pl.ds(hpos(h) * HP, DP // 2), :] for ct in range(3 * E // 128)], axis=1)
                qkv[h] = _dot(hl, pltpu.bitcast(w, _BF16))

            def stage_s(h):
                q = qkv[h][:, :E]
                k = qkv[h][:, E:2 * E].astype(_BF16)
                sc = jnp.where(mask, _dot_nt(q, k) * scale, -1e9)
                e = jnp.exp(sc - jnp.max(sc, axis=1, keepdims=True))
                pp[h] = e / jnp.sum(e, axis=1, keepdims=True)

            def stage_p(h):
                o_s[:, h * E:(h + 1) * E] = _dot(pp[h], qkv[h][:, 2 * E:].astype(_BF16))

            def stage_o(g):
                acc.append(_dot(o_s[:, g * G * E:(g + 1) * G * E],
                                pltpu.bitcast(wo[pl.ds(g * G * (E // 2), G * (E // 2)), :], _BF16)))

            todo = list(range(H // G))
            for t in range(H + D2):
                if t < H:
                    stage_q(t)
                if 0 <= t - D1 < H:
                    stage_s(t - D1)
                if 0 <= t - D2 < H:
                    stage_p(t - D2)
                if t >= H - 1 and todo and (todo[0] + 1) * G - 1 <= t - D2:
                    stage_o(todo.pop(0))
            while todo:
                stage_o(todo.pop(0))
            a = functools.reduce(lambda u, v: u + v, acc)
            out_s[rows, :] = a[M:, :].astype(_BF16)

            if NST == n_seg:
                @pl.when(jnp.logical_and((s + 1) % (OC // SEG) == 0, s + 1 < n_seg))
                def _():
                    flush((s + 1) // (OC // SEG) - 1)
            return a[:M, :]

        m0 = jnp.concatenate([mem0_s[...].astype(_F32), jnp.zeros((M, DP - D), _F32)], axis=1)
        with jax.named_scope("steps"):
            jax.lax.fori_loop(0, NST, step, m0, unroll=int("1"))
        with jax.named_scope("final"):
            flush(S // OC - 1)
            if NST == n_seg:
                pltpu.make_async_copy(outt_s, outt_hbm, osem).wait()
            else:
                pltpu.make_async_copy(outt_s.at[:, pl.ds(0, OC)], outt_hbm.at[:, pl.ds(0, OC)], osem).wait()

    return kernel


@functools.partial(jax.jit, static_argnames=("A_seg_len",))
def pallas_parallel_sum__memory_aug_recurrent_mem_tr__dense_activation_silu__prompt_kernel(
    A_x, A_mem0, A_Wq, A_Wk, A_Wv, A_Wo, A_seg_len, B_x, B_w1, B_w2,
):
    del B_x
    B, S, D = A_x.shape
    M = A_mem0.shape[1]
    _, H, E = A_Wq.shape
    F = B_w1.shape[1]
    SEG = int(A_seg_len)
    DP = -(-D // 128) * 128
    assert B == 1 and S % SEG == 0 and S % 512 == 0
    L = M + SEG
    kernel = _make_kernel(S, D, DP, H, E, M, SEG, F)
    hbm = pl.BlockSpec(memory_space=pltpu.HBM)
    out_t = pl.pallas_call(
        kernel,
        out_shape=pltpu.HBM((D, S), A_x.dtype),
        in_specs=[hbm] * 8,
        out_specs=hbm,
        scratch_shapes=[
            pltpu.VMEM((DP, S), _BF16),
            pltpu.VMEM((M, D), _BF16),
            pltpu.VMEM((3 * (E // 128), D * H, 128), _BF16),
            pltpu.VMEM((H * D, E), _BF16),
            pltpu.VMEM((D, F), _BF16),
            pltpu.VMEM((D, F), _BF16),
            pltpu.VMEM((S, DP), _F32),
            pltpu.VMEM((D, S), _F32),
            pltpu.VMEM((3 * E // 128, H * (DP // 2 + 8), 128), _U32),
            pltpu.VMEM((H * E // 2, DP), _U32),
            pltpu.VMEM((DP // 2, F), _U32),
            pltpu.VMEM((L, H * E), _F32),
            pltpu.VMEM((S, DP), _BF16),
            pltpu.VMEM((D, S), _BF16),
            pltpu.VMEM((256, F), _BF16),
            pltpu.VMEM((8, 128), _U32),
            pltpu.SemaphoreType.DMA((13,)),
            pltpu.SemaphoreType.DMA(()),
        ],
        compiler_params=pltpu.CompilerParams(vmem_limit_bytes=110 * 1024 * 1024),
    )(
        A_x.reshape(S, D).T, A_mem0.reshape(M, D),
        A_Wq.reshape(D * H, E), A_Wk.reshape(D * H, E), A_Wv.reshape(D * H, E),
        A_Wo.transpose(0, 2, 1).reshape(H * D, E), B_w1, B_w2.T,
    )
    return out_t.T.reshape(B, S, D)
```

```python
import functools

import jax
import jax.numpy as jnp
import numpy as np
from jax.experimental import pallas as pl
from jax.experimental.pallas import tpu as pltpu

_F32 = jnp.float32
_BF16 = jnp.bfloat16
_U32 = jnp.uint32


def _dot(a, b):
    return jax.lax.dot_general(a, b, (((1,), (0,)), ((), ())), preferred_element_type=_F32)


def _dot_nt(a, b):
    return jax.lax.dot_general(a, b, (((1,), (1,)), ((), ())), preferred_element_type=_F32)


def _aligned(i, n):
    return i if isinstance(i, int) else pl.multiple_of(i, n)


def _make_kernel(S, D, DP, H, E, M, SEG, F):
    n_seg = S // SEG
    HP = DP // 2 + 8
    hpos = lambda h: (h % 2) * (H // 2) + h // 2
    L = M + SEG
    FB = 256
    OC = 512
    CW = 256
    NB = S // FB
    NBB = 3
    scale = float(E) ** -0.5
    NST = int(n_seg)
    D1, D2 = int("2"), int("6")
    GL = [int(c, 36) for c in "22222222"]
    Z0 = int("0"); SZ = int("0")
    PZD = int("-1"); PZK = int("0")

    def kernel(xt_hbm, mem_hbm, wq_hbm, wk_hbm, wv_hbm, wot_hbm, w1_hbm, w2t_hbm, outt_hbm,
               xt, mem0_s, raw_w, raw_o, raw_1, w2t,
               xn, baset, wqkv, u_s, w1, out_s, outt_s, act_s, zero_s, sems, osem):
        cp_x0 = pltpu.make_async_copy(xt_hbm.at[:, pl.ds(0, FB)], xt.at[pl.ds(0, D), pl.ds(0, FB)], sems.at[0])
        cp_x1 = pltpu.make_async_copy(xt_hbm.at[:, pl.ds(FB, FB)], xt.at[pl.ds(0, D), pl.ds(FB, FB)], sems.at[11])
        cp_x2 = pltpu.make_async_copy(xt_hbm.at[:, pl.ds(2 * FB, S - 2 * FB)],
                                      xt.at[pl.ds(0, D), pl.ds(2 * FB, S - 2 * FB)], sems.at[12])
        cp_1 = pltpu.make_async_copy(w1_hbm, raw_1, sems.at[1])
        cp_2 = pltpu.make_async_copy(w2t_hbm, w2t, sems.at[2])
        cp_m = pltpu.make_async_copy(mem_hbm, mem0_s, sems.at[3])
        cp_att = []
        for i, src in enumerate((wq_hbm, wk_hbm, wv_hbm)):
            for ec in range(E // 128):
                cp_att.append(pltpu.make_async_copy(
                    src.at[:, pl.ds(ec * 128, 128)], raw_w.at[i * (E // 128) + ec], sems.at[4 + 2 * i + ec]))
        cp_att.append(pltpu.make_async_copy(wot_hbm, raw_o, sems.at[10]))
        DMAO = "1"
        for c in [cp_x0, cp_1, cp_2, cp_x1, cp_x2, cp_m] + (cp_att if DMAO == "0" else []):
            c.start()

        xt[pl.ds(D, DP - D), :] = jnp.zeros((DP - D, S), _BF16)
        for h in range(H):
            wqkv[:, pl.ds(h * HP + D // 2, (DP - D) // 2), :] = jnp.zeros((3 * E // 128, (DP - D) // 2, 128), _U32)
        w1[pl.ds(D // 2, (DP - D) // 2), :] = jnp.zeros(((DP - D) // 2, F), _U32)
        u_s[:, pl.ds(D // 2, (DP - D) // 2), :] = jnp.zeros((u_s.shape[0], (DP - D) // 2, 128), _U32)
        zero_s[...] = jnp.zeros((8, 128), _U32)
        lane = jax.lax.broadcasted_iota(jnp.int32, (FB, DP), 1)

        def layer_norm(i):
            r = _aligned(i * FB, FB)
            xf = xt[:, pl.ds(r, FB)].T.astype(_F32)
            mu = jnp.sum(xf, axis=1, keepdims=True) * (1.0 / D)
            c = jnp.where(lane < D, xf - mu, 0.0)
            var = jnp.sum(c * c, axis=1, keepdims=True) * (1.0 / D)
            xn[pl.ds(r, FB), :] = c * jax.lax.rsqrt(var + 1e-5)

        def xpose8(A):
            sub = jax.lax.broadcasted_iota(jnp.int32, A[0].shape, 0)
            A = list(A)
            for k in (4, 2, 1):
                m = (sub & k) != 0
                B = list(A)
                for i in range(8):
                    if i & k == 0:
                        B[i] = jnp.where(m, pltpu.roll(A[i + k], k, 0), A[i])
                        B[i + k] = jnp.where(m, A[i + k], pltpu.roll(A[i], 8 - k, 0))
                A = B
            return A

        def retile_qkv(j, zero):
            ru = raw_w.bitcast(_U32)
            dep = zero
            RT = "st"
            for ec in range(E // 128):
                jj = j * (E // 128) + ec
                for g in range(D // 16):
                    if RT == "st":
                        for i in range(8):
                            ev = ru[jj, pl.ds((16 * g + 2 * i) * 8, 8), :] | dep
                            od = ru[jj, pl.ds((16 * g + 2 * i + 1) * 8, 8), :] | dep
                            lo = (ev & _U32(0xFFFF)) | (od << 16)
                            last = (ev >> 16) | (od & _U32(0xFFFF0000))
                            wqkv[jj, pl.ds(8 * g + i, H // 2, stride=HP), :] = lo
                            wqkv[jj, pl.ds((H // 2) * HP + 8 * g + i, H // 2, stride=HP), :] = last
                    else:
                        ev = xpose8([ru[jj, pl.ds((16 * g + 2 * i) * 8, 8), :] | dep for i in range(8)])
                        od = xpose8([ru[jj, pl.ds((16 * g + 2 * i + 1) * 8, 8), :] | dep for i in range(8)])
                        for p in range(H // 2):
                            wqkv[jj, pl.ds(hpos(2 * p) * HP + g * 8, 8), :] = (ev[p] & _U32(0xFFFF)) | (od[p] << 16)
                            last = (ev[p] >> 16) | (od[p] & _U32(0xFFFF0000))
                            wqkv[jj, pl.ds(hpos(2 * p + 1) * HP + g * 8, 8), :] = last
                    if "1" == "1":
                        dep = pltpu.roll(last & zero, 1, 1)

        NU = 2 * DP // 128 - 1

        def fuse_vo(p, _):
            def wv(pos):
                rows = pl.ds(pl.multiple_of(pos * HP, 8), D // 2)
                tiles = [wqkv[2 * (E // 128) + ec, rows, :] for ec in range(E // 128)]
                return pltpu.bitcast(jnp.concatenate(tiles, axis=1), _BF16)
            r0 = pl.multiple_of(2 * p * D, 64)
            pad = jnp.zeros((DP - D, E), _BF16)
            cut = D // 128 * 128
            even = _dot_nt(wv(p), jnp.concatenate([raw_o[pl.ds(r0, D), :], pad], axis=0))
            odd = _dot_nt(wv(H // 2 + p), jnp.concatenate(
                [pad, raw_o[pl.ds(r0 + D + cut, D - cut), :], raw_o[pl.ds(r0 + D, cut), :]], axis=0))
            nt = DP // 128
            tiles = [even[:, 128 * j:128 * (j + 1)] for j in range(nt - 1)]
            tiles.append(even[:, 128 * (nt - 1):] + odd[:, :128])
            tiles += [odd[:, 128 * j:128 * (j + 1)] for j in range(1, nt)]
            for j, t in enumerate(tiles):
                u_s[p * NU + j, pl.ds(0, D // 2), :] = pltpu.bitcast(t.astype(_BF16), _U32)
            return _

        def ffn_up(i, after_load=None):
            xb = xn[pl.ds(_aligned(i * FB, FB), FB), :]
            if after_load is not None:
                after_load()
            for c in range(F // CW):
                half = _dot(xb, pltpu.bitcast(w1[:, pl.ds(c * CW, CW)], _BF16)) * 0.5
                act_s[:, pl.ds(c * CW, CW)] = (half * jnp.tanh(half) + half).astype(_BF16)

        def ffn_down(i, between=None):
            cols = pl.ds(_aligned(i * FB, FB), FB)
            NC = int("2")
            w = D // NC
            for n in range(NC):
                rows = pl.ds(n * w, w)
                yt = _dot_nt(w2t[rows, :], act_s[...])
                baset[rows, cols] = yt + xt[rows, cols].astype(_F32)
                if between is not None:
                    between(n)

        with jax.named_scope("first"):
            cp_x0.wait()
            layer_norm(0)
            cp_1.wait()

            def pack_w1(i, _):
                w1[pl.ds(pl.multiple_of(i * 32, 32), 32), :] = pltpu.bitcast(
                    raw_1[pl.ds(pl.multiple_of(i * 64, 64), 64), :], _U32)
                return _
            jax.lax.fori_loop(0, D // 64, pack_w1, 0)
            if DMAO == "1":
                for c in cp_att:
                    c.start()
            ffn_up(0)
        with jax.named_scope("wait_w2"):
            cp_2.wait()
            cp_x1.wait()
            if DMAO == "2":
                for c in cp_att:
                    c.start()
        with jax.named_scope("second"):
            ffn_down(0)
            layer_norm(1)

        cp_x2.wait()

        def ffn_a(i, _):
            LP = "2"
            if LP == "0":
                ffn_up(i, lambda: layer_norm(i + 1))
                ffn_down(i)
            elif LP == "1":
                ffn_up(i)
                layer_norm(i + 1)
                ffn_down(i)
            else:
                ffn_up(i)
                ffn_down(i)
                layer_norm(i + 1)
            return _
        with jax.named_scope("loopA"):
            jax.lax.fori_loop(1, NB - NBB, ffn_a, 0, unroll=int("1"))

        with jax.named_scope("wait_att"):
            for c in cp_att:
                c.wait()
            cp_m.wait()

        def ffn_b(j, _):
            if "1" == "1":
                retile_qkv(j, zero_s[...])
            LP = "2"
            lnb = lambda: layer_norm(jnp.minimum(j + (NB - NBB) + 1, NB - 1))
            ffn_up(j + NB - NBB, lnb if LP == "0" else None)
            if LP == "1":
                lnb()
            ffn_down(j + NB - NBB)
            if LP == "2":
                lnb()
            return _
        with jax.named_scope("loopB"):
            jax.lax.fori_loop(0, NBB, ffn_b, 0, unroll=int("3"))

        with jax.named_scope("fuse_vo"):
            jax.lax.fori_loop(0, H // 2, fuse_vo, 0, unroll=int("8"))

        row = jax.lax.broadcasted_iota(jnp.int32, (L, L), 0)
        col = jax.lax.broadcasted_iota(jnp.int32, (L, L), 1)
        mask = (row < M) | (row >= col)
        lane128 = jax.lax.broadcasted_iota(jnp.int32, (L, 128), 1)

        def flush(c):
            cols = pl.ds(_aligned(c * OC, OC), OC)
            at = out_s[cols, :].T
            outt_s[:, cols] = (baset[:, cols] + at[:D].astype(_F32)).astype(_BF16)
            pltpu.make_async_copy(outt_s.at[:, cols], outt_hbm.at[:, cols], osem).start()

        def step(s, mem):
            rows = pl.ds(pl.multiple_of(s * SEG, SEG), SEG)
            hl = jnp.concatenate([mem, xn[rows, :]], axis=0)
            qkv, pp, zz, acc = {}, {}, {}, [None]
            NKT = H * L // 128

            def stage_q(h):
                w = jnp.concatenate([wqkv[ct, pl.ds(hpos(h) * HP, DP // 2), :] for ct in range(2 * E // 128)], axis=1)
                qkv[h] = _dot(hl, pltpu.bitcast(w, _BF16))

            def stage_s(h):
                q = qkv[h][:, :E]
                k = qkv[h][:, E:].astype(_BF16)
                sc = jnp.where(mask, _dot_nt(q, k) * scale, -1e9)
                e = jnp.exp(sc - jnp.max(sc, axis=1, keepdims=True))
                p = e / jnp.sum(e, axis=1, keepdims=True)
                p = jnp.concatenate([p, jnp.zeros((L, 128 - L), _F32)], axis=1)
                off = (h * L) % 128
                pp[h] = pltpu.roll(p, off, 1) if off else p

            def stage_z(p):
                nt = NU // 2
                tails = _dot(hl, pltpu.bitcast(u_s[p * NU + nt], _BF16))
                odd_tail = pltpu.roll(tails, 64, 1)
                w = jnp.concatenate([u_s[p * NU + j] for j in range(NU) if j != nt], axis=1)
                z = _dot(hl, pltpu.bitcast(w, _BF16))
                zz[2 * p] = jnp.concatenate([z[:, :128 * nt], tails], axis=1)
                zz[2 * p + 1] = jnp.concatenate([z[:, 128 * nt:], odd_tail], axis=1)

            def tile_heads(t):
                return [h for h in range(H) if h * L < (t + 1) * 128 and (h + 1) * L > t * 128]

            def stage_o(t):
                pt = None
                for h in tile_heads(t):
                    lo, hi = max(h * L - t * 128, 0), min((h + 1) * L - t * 128, 128)
                    if hi - lo < L:
                        piece = jnp.where((lane128 >= lo) & (lane128 < hi), pp[h], 0.0)
                    else:
                        piece = pp[h]
                    pt = piece if pt is None else pt + piece
                hs = tile_heads(t)
                zt = jnp.concatenate([zz[h] for h in hs], axis=0)
                r0 = t * 128 - hs[0] * L
                c = _dot(pt, zt[r0:r0 + 128].astype(_BF16))
                acc[0] = c if acc[0] is None else acc[0] + c

            for t in range(H):
                stage_q(t)
                if t >= D1:
                    stage_s(t - D1)
            ns = H - D1
            zord = [(p + Z0) % (H // 2) for p in range(H // 2)]
            for n, p in enumerate(zord):
                stage_z(p)
                if ns < H and n >= SZ:
                    stage_s(ns)
                    ns += 1
            while ns < H:
                stage_s(ns)
                ns += 1
            for t in sorted(range(NKT), key=lambda t: max(zord.index(h // 2) for h in tile_heads(t))):
                stage_o(t)
            a = acc[0]
            out_s[rows, :] = a[M:, :].astype(_BF16)

            return a[:M, :]

        m0 = jnp.concatenate([mem0_s[...].astype(_F32), jnp.zeros((M, DP - D), _F32)], axis=1)
        SPC = OC // SEG

        def chunk(c, mem):
            mem = jax.lax.fori_loop(0, SPC, lambda i, m: step(c * SPC + i, m), mem,
                                    unroll=int("2"))
            flush(c)
            return mem
        with jax.named_scope("steps"):
            jax.lax.fori_loop(0, NST // SPC, chunk, m0)
        with jax.named_scope("final"):
            n = NST // SPC * OC
            pltpu.make_async_copy(outt_s.at[:, pl.ds(0, n)], outt_hbm.at[:, pl.ds(0, n)], osem).wait()

    return kernel


@functools.partial(jax.jit, static_argnames=("A_seg_len",))
def pallas_parallel_sum__memory_aug_recurrent_mem_tr__dense_activation_silu__prompt_kernel(
    A_x, A_mem0, A_Wq, A_Wk, A_Wv, A_Wo, A_seg_len, B_x, B_w1, B_w2,
):
    del B_x
    B, S, D = A_x.shape
    M = A_mem0.shape[1]
    _, H, E = A_Wq.shape
    F = B_w1.shape[1]
    SEG = int(A_seg_len)
    DP = -(-D // 128) * 128
    assert B == 1 and S % SEG == 0 and S % 512 == 0
    L = M + SEG
    kernel = _make_kernel(S, D, DP, H, E, M, SEG, F)
    hbm = pl.BlockSpec(memory_space=pltpu.HBM)
    out_t = pl.pallas_call(
        kernel,
        out_shape=pltpu.HBM((D, S), A_x.dtype),
        in_specs=[hbm] * 8,
        out_specs=hbm,
        scratch_shapes=[
            pltpu.VMEM((DP, S), _BF16),
            pltpu.VMEM((M, D), _BF16),
            pltpu.VMEM((3 * (E // 128), D * H, 128), _BF16),
            pltpu.VMEM((H * D, E), _BF16),
            pltpu.VMEM((D, F), _BF16),
            pltpu.VMEM((D, F), _BF16),
            pltpu.VMEM((S, DP), _F32),
            pltpu.VMEM((D, S), _F32),
            pltpu.VMEM((3 * E // 128, H * (DP // 2 + 8), 128), _U32),
            pltpu.VMEM((H // 2 * (2 * DP // 128 - 1), DP // 2, 128), _U32),
            pltpu.VMEM((DP // 2, F), _U32),
            pltpu.VMEM((S, DP), _BF16),
            pltpu.VMEM((D, S), _BF16),
            pltpu.VMEM((256, F), _BF16),
            pltpu.VMEM((8, 128), _U32),
            pltpu.SemaphoreType.DMA((13,)),
            pltpu.SemaphoreType.DMA(()),
        ],
        compiler_params=pltpu.CompilerParams(vmem_limit_bytes=110 * 1024 * 1024),
    )(
        A_x.reshape(S, D).T, A_mem0.reshape(M, D),
        A_Wq.reshape(D * H, E), A_Wk.reshape(D * H, E), A_Wv.reshape(D * H, E),
        A_Wo.transpose(0, 2, 1).reshape(H * D, E), B_w1, B_w2.T,
    )
    return out_t.T.reshape(B, S, D)
```

```python
import functools

import jax
import jax.numpy as jnp
import numpy as np
from jax.experimental import pallas as pl
from jax.experimental.pallas import tpu as pltpu

_F32 = jnp.float32
_BF16 = jnp.bfloat16
_U32 = jnp.uint32


def _dot(a, b):
    return jax.lax.dot_general(a, b, (((1,), (0,)), ((), ())), preferred_element_type=_F32)


def _dot_nt(a, b):
    return jax.lax.dot_general(a, b, (((1,), (1,)), ((), ())), preferred_element_type=_F32)


def _aligned(i, n):
    return i if isinstance(i, int) else pl.multiple_of(i, n)


def _make_kernel(S, D, DP, H, E, M, SEG, F):
    n_seg = S // SEG
    HP = DP // 2 + 8
    hpos = lambda h: (h % 2) * (H // 2) + h // 2
    L = M + SEG
    FB = 256
    CW = 256
    NB = S // FB
    NBB = 3
    scale = float(E) ** -0.5
    NST = int(n_seg)
    D1, D2 = int("2"), int("6")
    GL = [int(c, 36) for c in "22222222"]
    JP = int("4"); JU = int("1")
    Z0 = int("0"); SZ = int("0")
    PZD = int("-1"); PZK = int("0")

    def kernel(xt_hbm, mem_hbm, wq_hbm, wk_hbm, wv_hbm, wot_hbm, w1_hbm, w2t_hbm, outt_hbm,
               xt, mem0_s, raw_w, raw_o, w2t,
               xn, baset, wqkv, u_s, w1, out_s, outt_s, act_s, zero_s, sems, osem):
        cp_x0 = pltpu.make_async_copy(xt_hbm.at[:, pl.ds(0, FB)], xt.at[pl.ds(0, D), pl.ds(0, FB)], sems.at[0])
        cp_x1 = pltpu.make_async_copy(xt_hbm.at[:, pl.ds(FB, FB)], xt.at[pl.ds(0, D), pl.ds(FB, FB)], sems.at[11])
        cp_x2 = pltpu.make_async_copy(xt_hbm.at[:, pl.ds(2 * FB, FB)], xt.at[pl.ds(0, D), pl.ds(2 * FB, FB)], sems.at[12])
        cp_x3 = pltpu.make_async_copy(xt_hbm.at[:, pl.ds(3 * FB, S - 3 * FB)],
                                      xt.at[pl.ds(0, D), pl.ds(3 * FB, S - 3 * FB)], sems.at[1])
        W1S = [int(c) for c in "0246"] + [F // CW]
        W1P = tuple(zip(W1S[:-1], W1S[1:]))
        cp_1 = [pltpu.make_async_copy(w1_hbm.at[:, pl.ds(a * CW, (b - a) * CW)],
                                      w1.at[pl.ds(0, D), pl.ds(a * CW, (b - a) * CW)], sems.at[13 + n])
                for n, (a, b) in enumerate(W1P)]
        cp_2 = pltpu.make_async_copy(w2t_hbm, w2t, sems.at[2])
        cp_m = pltpu.make_async_copy(mem_hbm, mem0_s, sems.at[3])
        cp_att = []
        for i, src in enumerate((wq_hbm, wk_hbm, wv_hbm)):
            for ec in range(E // 128):
                cp_att.append(pltpu.make_async_copy(
                    src.at[:, pl.ds(ec * 128, 128)], raw_w.at[i * (E // 128) + ec], sems.at[4 + 2 * i + ec]))
        cp_att.append(pltpu.make_async_copy(wot_hbm, raw_o, sems.at[10]))
        for c in [cp_x0] + cp_1[:-1] + [cp_x1, cp_1[-1], cp_2, cp_x2, cp_x3, cp_m] + cp_att:
            c.start()

        xt[pl.ds(D, DP - D), :] = jnp.zeros((DP - D, S), _BF16)
        for h in range(H):
            wqkv[:, pl.ds(h * HP + D // 2, (DP - D) // 2), :] = jnp.zeros((3 * E // 128, (DP - D) // 2, 128), _U32)
        w1[pl.ds(D, DP - D), :] = jnp.zeros((DP - D, F), _BF16)
        u_s[:, pl.ds(D // 2, (DP - D) // 2), :] = jnp.zeros((u_s.shape[0], (DP - D) // 2, 128), _U32)
        zero_s[...] = jnp.zeros((8, 128), _U32)
        baset[pl.ds(D, DP - D), :] = jnp.zeros((DP - D, S), _F32)
        out_s[pl.ds(0, 128), :] = jnp.zeros((128, DP), _BF16)
        lane = jax.lax.broadcasted_iota(jnp.int32, (FB, DP), 1)

        def layer_norm(i):
            r = _aligned(i * FB, FB)
            xf = xt[:, pl.ds(r, FB)].T.astype(_F32)
            mu = jnp.sum(xf, axis=1, keepdims=True) * (1.0 / D)
            c = jnp.where(lane < D, xf - mu, 0.0)
            var = jnp.sum(c * c, axis=1, keepdims=True) * (1.0 / D)
            xn[pl.ds(r, FB), :] = c * jax.lax.rsqrt(var + 1e-5)

        def xpose8(A):
            sub = jax.lax.broadcasted_iota(jnp.int32, A[0].shape, 0)
            A = list(A)
            for k in (4, 2, 1):
                m = (sub & k) != 0
                B = list(A)
                for i in range(8):
                    if i & k == 0:
                        B[i] = jnp.where(m, pltpu.roll(A[i + k], k, 0), A[i])
                        B[i + k] = jnp.where(m, A[i + k], pltpu.roll(A[i], 8 - k, 0))
                A = B
            return A

        def retile_qkv(j, zero):
            ru = raw_w.bitcast(_U32)
            dep = zero
            RT = "st"
            for ec in range(E // 128):
                jj = j * (E // 128) + ec
                for g in range(D // 16):
                    if RT == "st":
                        for i in range(8):
                            ev = ru[jj, pl.ds((16 * g + 2 * i) * 8, 8), :] | dep
                            od = ru[jj, pl.ds((16 * g + 2 * i + 1) * 8, 8), :] | dep
                            lo = (ev & _U32(0xFFFF)) | (od << 16)
                            last = (ev >> 16) | (od & _U32(0xFFFF0000))
                            wqkv[jj, pl.ds(8 * g + i, H // 2, stride=HP), :] = lo
                            wqkv[jj, pl.ds((H // 2) * HP + 8 * g + i, H // 2, stride=HP), :] = last
                    else:
                        ev = xpose8([ru[jj, pl.ds((16 * g + 2 * i) * 8, 8), :] | dep for i in range(8)])
                        od = xpose8([ru[jj, pl.ds((16 * g + 2 * i + 1) * 8, 8), :] | dep for i in range(8)])
                        for p in range(H // 2):
                            wqkv[jj, pl.ds(hpos(2 * p) * HP + g * 8, 8), :] = (ev[p] & _U32(0xFFFF)) | (od[p] << 16)
                            last = (ev[p] >> 16) | (od[p] & _U32(0xFFFF0000))
                            wqkv[jj, pl.ds(hpos(2 * p + 1) * HP + g * 8, 8), :] = last
                    if "1" == "1":
                        dep = pltpu.roll(last & zero, 1, 1)

        NU = 2 * DP // 128 - 1

        def fuse_vo(p, _):
            def wv(pos):
                rows = pl.ds(pl.multiple_of(pos * HP, 8), D // 2)
                tiles = [wqkv[2 * (E // 128) + ec, rows, :] for ec in range(E // 128)]
                return pltpu.bitcast(jnp.concatenate(tiles, axis=1), _BF16)
            r0 = pl.multiple_of(2 * p * D, 64)
            pad = jnp.zeros((DP - D, E), _BF16)
            cut = D // 128 * 128
            even = _dot_nt(wv(p), jnp.concatenate([raw_o[pl.ds(r0, D), :], pad], axis=0))
            odd = _dot_nt(wv(H // 2 + p), jnp.concatenate(
                [pad, raw_o[pl.ds(r0 + D + cut, D - cut), :], raw_o[pl.ds(r0 + D, cut), :]], axis=0))
            nt = DP // 128
            tiles = [even[:, 128 * j:128 * (j + 1)] for j in range(nt - 1)]
            tiles.append(even[:, 128 * (nt - 1):] + odd[:, :128])
            tiles += [odd[:, 128 * j:128 * (j + 1)] for j in range(1, nt)]
            for j, t in enumerate(tiles):
                u_s[p * NU + j, pl.ds(0, D // 2), :] = pltpu.bitcast(t.astype(_BF16), _U32)
            return _

        def ffn_up(i, chunks=None):
            xb = xn[pl.ds(_aligned(i * FB, FB), FB), :]
            for c in chunks if chunks is not None else range(F // CW):
                half = _dot(xb, w1[:, pl.ds(c * CW, CW)]) * 0.5
                act_s[i % 2, :, pl.ds(c * CW, CW)] = (half * jnp.tanh(half) + half).astype(_BF16)

        def ffn_down(i):
            cols = pl.ds(_aligned(i * FB, FB), FB)
            w = D // 2
            for n in range(2):
                rows = pl.ds(n * w, w)
                baset[rows, cols] = _dot_nt(w2t[rows, :], act_s[i % 2]) + xt[rows, cols].astype(_F32)

        def ffn(i):
            ffn_up(i + 1)
            ffn_down(i)
            if not isinstance(i, int) or i + 2 < NB:
                layer_norm(i + 2)

        with jax.named_scope("first"):
            cp_x0.wait()
            layer_norm(0)
            for n, (c, (a, b)) in enumerate(zip(cp_1, W1P)):
                c.wait()
                if n == len(W1P) - 1:
                    cp_x1.wait()
                ffn_up(0, range(a, b))
            layer_norm(1)
            ffn_up(1)
        with jax.named_scope("w2wait"):
            cp_2.wait()
        with jax.named_scope("x2wait"):
            cp_x2.wait()
        with jax.named_scope("second"):
            ffn_down(0)
            layer_norm(2)
        with jax.named_scope("x3wait"):
            cp_x3.wait()
        with jax.named_scope("loopA"):
            def ffn_a(i, _):
                ffn(i)
                return _
            jax.lax.fori_loop(1, NB - 1 - NBB, ffn_a, 0, unroll=int("1"))
        with jax.named_scope("loopB"):
            for j in range(NBB):
                for c in cp_att[j * (E // 128):(j + 1) * (E // 128)]:
                    c.wait()
                retile_qkv(j, zero_s[...])
                ffn(NB - 1 - NBB + j)
            cp_att[-1].wait()
            ffn_down(NB - 1)

        with jax.named_scope("fuse_vo"):
            jax.lax.fori_loop(0, H // 2, fuse_vo, 0, unroll=int("8"))

        cp_m.wait()
        row = jax.lax.broadcasted_iota(jnp.int32, (L, L), 0)
        col = jax.lax.broadcasted_iota(jnp.int32, (L, L), 1)
        mask = (row < M) | (row >= col)
        lane128 = jax.lax.broadcasted_iota(jnp.int32, (L, 128), 1)

        def flush(start, size):
            cols = pl.ds(start, size)
            at = out_s[cols, :].T
            outt_s[pl.ds(0, D), cols] = (baset[pl.ds(0, D), cols] + at[:D].astype(_F32)).astype(_BF16)
            pltpu.make_async_copy(outt_s.at[pl.ds(0, D), cols], outt_hbm.at[:, cols], osem).start()

        def w_qk(h):
            tiles = [wqkv[ct, pl.ds(hpos(h) * HP, DP // 2), :] for ct in range(2 * E // 128)]
            return pltpu.bitcast(jnp.concatenate(tiles, axis=1), _BF16)

        def step(s, mem, ahead, job=None):
            rows = pl.ds(pl.multiple_of(s * SEG, SEG), SEG)
            hl = jnp.concatenate([mem, xn[rows, :]], axis=0)
            qkv, pp, zz, acc = {}, {}, {}, [None]
            NKT = H * L // 128

            def stage_q(h):
                if h in ahead:
                    qkv[h] = jnp.concatenate([_dot(mem, w_qk(h)), ahead[h]], axis=0)
                else:
                    qkv[h] = _dot(hl, w_qk(h))

            def stage_s(h):
                q = qkv[h][:, :E]
                k = qkv[h][:, E:].astype(_BF16)
                sc = jnp.where(mask, _dot_nt(q, k) * scale, -1e9)
                e = jnp.exp(sc - jnp.max(sc, axis=1, keepdims=True))
                p = e / jnp.sum(e, axis=1, keepdims=True)
                p = jnp.concatenate([p, jnp.zeros((L, 128 - L), _F32)], axis=1)
                off = (h * L) % 128
                pp[h] = pltpu.roll(p, off, 1) if off else p

            def stage_z(p):
                nt = NU // 2
                tails = _dot(hl, pltpu.bitcast(u_s[p * NU + nt], _BF16))
                odd_tail = pltpu.roll(tails, 64, 1)
                w = jnp.concatenate([u_s[p * NU + j] for j in range(NU) if j != nt], axis=1)
                z = _dot(hl, pltpu.bitcast(w, _BF16))
                zz[2 * p] = jnp.concatenate([z[:, :128 * nt], tails], axis=1)
                zz[2 * p + 1] = jnp.concatenate([z[:, 128 * nt:], odd_tail], axis=1)

            def tile_heads(t):
                return [h for h in range(H) if h * L < (t + 1) * 128 and (h + 1) * L > t * 128]

            def stage_o(t):
                pt = None
                for h in tile_heads(t):
                    lo, hi = max(h * L - t * 128, 0), min((h + 1) * L - t * 128, 128)
                    if hi - lo < L:
                        piece = jnp.where((lane128 >= lo) & (lane128 < hi), pp[h], 0.0)
                    else:
                        piece = pp[h]
                    pt = piece if pt is None else pt + piece
                hs = tile_heads(t)
                zt = jnp.concatenate([zz[h] for h in hs], axis=0)
                r0 = t * 128 - hs[0] * L
                c = _dot(pt, zt[r0:r0 + 128].astype(_BF16))
                acc[0] = c if acc[0] is None else acc[0] + c

            for t in range(H):
                stage_q(t)
                if t >= D1:
                    stage_s(t - D1)
            ns = H - D1
            zord = [(p + Z0) % (H // 2) for p in range(H // 2)]
            for n, p in enumerate(zord):
                stage_z(p)
                if job is not None and n == JP:
                    job(zz[2 * p][:8, :128])
                if ns < H and n >= SZ:
                    stage_s(ns)
                    ns += 1
            while ns < H:
                stage_s(ns)
                ns += 1
            for t in sorted(range(NKT), key=lambda t: max(zord.index(h // 2) for h in tile_heads(t))):
                stage_o(t)
            a = acc[0]
            out_s[rows, :] = a[M:, :].astype(_BF16)

            return a[:M, :]

        m0 = jnp.concatenate([mem0_s[...].astype(_F32), jnp.zeros((M, DP - D), _F32)], axis=1)
        UNR = int("2")
        NAH = int("1")
        OC = int("640")
        n_full = (S - 1) // OC

        INC = "1" == "1"

        def out_job(it, pin):
            blk = jnp.maximum(it - 2, 0)
            tb = pl.multiple_of((blk // 2) * 128, 128)
            f0 = pl.multiple_of((blk % 2) * (DP // 2), DP // 2)
            zero = pltpu.bitcast(pin, _U32) & zero_s[...]
            a = pltpu.bitcast(out_s[pl.ds(tb, 128), pl.ds(f0, DP // 2)], _U32)
            a = pltpu.bitcast(a | jnp.tile(zero, (a.shape[0] // 8, a.shape[1] // 128)), _BF16)
            res = baset[pl.ds(f0, DP // 2), pl.ds(tb, 128)] + a.T.astype(_F32)
            outt_s[pl.ds(f0, DP // 2), pl.ds(tb, 128)] = res.astype(_BF16)

        def send(tb):
            cols = pl.ds(tb, 128)
            pltpu.make_async_copy(outt_s.at[pl.ds(0, D), cols], outt_hbm.at[:, cols], osem).start()

        def steps(it, mem):
            ahead = {}
            for u in range(UNR):
                s = it * UNR + u
                mem = step(s, mem, ahead, (lambda pin: out_job(it, pin)) if (INC and u == JU) else None)
                if u + 1 < UNR:
                    xs = xn[pl.ds(pl.multiple_of((s + 1) * SEG, SEG), SEG), :]
                    ahead = {h: _dot(xs, w_qk(h)) for h in range(NAH)}

            if INC:
                @pl.when(jnp.logical_and(it % 2 == 1, it >= 3))
                def _():
                    send(pl.multiple_of((it - 3) // 2 * 128, 128))
                return mem
            done = (it + 1) * (UNR * SEG)

            @pl.when(jnp.logical_and(done % OC == 0, done < S))
            def _():
                flush(pl.multiple_of(done - OC, 128), OC)
            return mem

        with jax.named_scope("steps"):
            jax.lax.fori_loop(0, n_seg // UNR, steps, m0)
        with jax.named_scope("final"):
            if INC:
                nit = n_seg // UNR
                for it in (nit, nit + 1):
                    out_job(it, jnp.zeros((8, 128), _F32))
                send(S - 128)
            else:
                flush(n_full * OC, S - n_full * OC)
            pltpu.make_async_copy(outt_s.at[pl.ds(0, D)], outt_hbm, osem).wait()

    return kernel


@functools.partial(jax.jit, static_argnames=("A_seg_len",))
def pallas_parallel_sum__memory_aug_recurrent_mem_tr__dense_activation_silu__prompt_kernel(
    A_x, A_mem0, A_Wq, A_Wk, A_Wv, A_Wo, A_seg_len, B_x, B_w1, B_w2,
):
    del B_x
    B, S, D = A_x.shape
    M = A_mem0.shape[1]
    _, H, E = A_Wq.shape
    F = B_w1.shape[1]
    SEG = int(A_seg_len)
    DP = -(-D // 128) * 128
    assert B == 1 and S % SEG == 0 and S % 512 == 0
    L = M + SEG
    kernel = _make_kernel(S, D, DP, H, E, M, SEG, F)
    hbm = pl.BlockSpec(memory_space=pltpu.HBM)
    out_t = pl.pallas_call(
        kernel,
        out_shape=pltpu.HBM((D, S), A_x.dtype),
        in_specs=[hbm] * 8,
        out_specs=hbm,
        scratch_shapes=[
            pltpu.VMEM((DP, S), _BF16),
            pltpu.VMEM((M, D), _BF16),
            pltpu.VMEM((3 * (E // 128), D * H, 128), _BF16),
            pltpu.VMEM((H * D, E), _BF16),
            pltpu.VMEM((D, F), _BF16),
            pltpu.VMEM((S, DP), _F32),
            pltpu.VMEM((DP, S), _F32),
            pltpu.VMEM((3 * E // 128, H * (DP // 2 + 8), 128), _U32),
            pltpu.VMEM((H // 2 * (2 * DP // 128 - 1), DP // 2, 128), _U32),
            pltpu.VMEM((DP, F), _BF16),
            pltpu.VMEM((S, DP), _BF16),
            pltpu.VMEM((DP, S), _BF16),
            pltpu.VMEM((2, 256, F), _BF16),
            pltpu.VMEM((8, 128), _U32),
            pltpu.SemaphoreType.DMA((20,)),
            pltpu.SemaphoreType.DMA(()),
        ],
        compiler_params=pltpu.CompilerParams(vmem_limit_bytes=110 * 1024 * 1024),
    )(
        A_x.reshape(S, D).T, A_mem0.reshape(M, D),
        A_Wq.reshape(D * H, E), A_Wk.reshape(D * H, E), A_Wv.reshape(D * H, E),
        A_Wo.transpose(0, 2, 1).reshape(H * D, E), B_w1, B_w2.T,
    )
    return out_t.T.reshape(B, S, D)
```

```python
import functools

import jax
import jax.numpy as jnp
import numpy as np
from jax.experimental import pallas as pl
from jax.experimental.pallas import tpu as pltpu

_F32 = jnp.float32
_BF16 = jnp.bfloat16
_U32 = jnp.uint32


def _dot(a, b):
    return jax.lax.dot_general(a, b, (((1,), (0,)), ((), ())), preferred_element_type=_F32)


def _dot_nt(a, b):
    return jax.lax.dot_general(a, b, (((1,), (1,)), ((), ())), preferred_element_type=_F32)


def _aligned(i, n):
    return i if isinstance(i, int) else pl.multiple_of(i, n)


def _make_kernel(S, D, DP, H, E, M, SEG, F):
    n_seg = S // SEG
    HP = DP // 2 + 8
    hpos = lambda h: (h % 2) * (H // 2) + h // 2
    L = M + SEG
    FB = 256
    CW = 256
    NB = S // FB
    scale = float(E) ** -0.5
    NST = int(n_seg)
    D1, D2 = int("2"), int("6")
    GL = [int(c, 36) for c in "22222222"]
    JP = int("4"); JU = int("1")
    Z0 = int("0"); SZ = int("0")
    PZD = int("-1"); PZK = int("0")

    def kernel(xt_hbm, mem_hbm, wq_hbm, wk_hbm, wv_hbm, wot_hbm, w1_hbm, w2t_hbm, outt_hbm,
               xt, mem0_s, raw_w, raw_o, w2t,
               xn, baset, wqkv, u_s, w1, out_s, outt_s, act_s, zero_s, sems, osem):
        cp_x0 = pltpu.make_async_copy(xt_hbm.at[:, pl.ds(0, FB)], xt.at[pl.ds(0, D), pl.ds(0, FB)], sems.at[0])
        cp_x1 = pltpu.make_async_copy(xt_hbm.at[:, pl.ds(FB, FB)], xt.at[pl.ds(0, D), pl.ds(FB, FB)], sems.at[11])
        cp_x2 = pltpu.make_async_copy(xt_hbm.at[:, pl.ds(2 * FB, FB)], xt.at[pl.ds(0, D), pl.ds(2 * FB, FB)], sems.at[12])
        cp_x3 = pltpu.make_async_copy(xt_hbm.at[:, pl.ds(3 * FB, S - 3 * FB)],
                                      xt.at[pl.ds(0, D), pl.ds(3 * FB, S - 3 * FB)], sems.at[1])
        W1S = [int(c) for c in "0246"] + [F // CW]
        W1P = tuple(zip(W1S[:-1], W1S[1:]))
        cp_1 = [pltpu.make_async_copy(w1_hbm.at[:, pl.ds(a * CW, (b - a) * CW)],
                                      w1.at[pl.ds(0, D), pl.ds(a * CW, (b - a) * CW)], sems.at[13 + n])
                for n, (a, b) in enumerate(W1P)]
        cp_2 = pltpu.make_async_copy(w2t_hbm, w2t, sems.at[2])
        cp_m = pltpu.make_async_copy(mem_hbm, mem0_s, sems.at[3])
        cp_att = []
        for i, src in enumerate((wq_hbm, wk_hbm, wv_hbm)):
            for ec in range(E // 128):
                cp_att.append(pltpu.make_async_copy(
                    src.at[:, pl.ds(ec * 128, 128)], raw_w.at[i * (E // 128) + ec], sems.at[4 + 2 * i + ec]))
        cp_att.append(pltpu.make_async_copy(wot_hbm, raw_o, sems.at[10]))
        for c in [cp_x0] + cp_1[:-1] + [cp_x1, cp_1[-1], cp_2, cp_x2, cp_x3, cp_m] + cp_att:
            c.start()

        xt[pl.ds(D, DP - D), :] = jnp.zeros((DP - D, S), _BF16)
        for h in range(H):
            wqkv[:, pl.ds(h * HP + D // 2, (DP - D) // 2), :] = jnp.zeros((3 * E // 128, (DP - D) // 2, 128), _U32)
        w1[pl.ds(D, DP - D), :] = jnp.zeros((DP - D, F), _BF16)
        u_s[:, pl.ds(D // 2, (DP - D) // 2), :] = jnp.zeros((u_s.shape[0], (DP - D) // 2, 128), _U32)
        zero_s[...] = jnp.zeros((8, 128), _U32)
        baset[pl.ds(D, DP - D), :] = jnp.zeros((DP - D, S), _F32)
        out_s[pl.ds(0, 128), :] = jnp.zeros((128, DP), _BF16)
        lane = jax.lax.broadcasted_iota(jnp.int32, (FB, DP), 1)

        def layer_norm(i):
            r = _aligned(i * FB, FB)
            xf = xt[:, pl.ds(r, FB)].T.astype(_F32)
            mu = jnp.sum(xf, axis=1, keepdims=True) * (1.0 / D)
            c = jnp.where(lane < D, xf - mu, 0.0)
            var = jnp.sum(c * c, axis=1, keepdims=True) * (1.0 / D)
            xn[pl.ds(r, FB), :] = c * jax.lax.rsqrt(var + 1e-5)

        def xpose8(A):
            sub = jax.lax.broadcasted_iota(jnp.int32, A[0].shape, 0)
            A = list(A)
            for k in (4, 2, 1):
                m = (sub & k) != 0
                B = list(A)
                for i in range(8):
                    if i & k == 0:
                        B[i] = jnp.where(m, pltpu.roll(A[i + k], k, 0), A[i])
                        B[i + k] = jnp.where(m, A[i + k], pltpu.roll(A[i], 8 - k, 0))
                A = B
            return A

        def retile(jj, zero):
            ru = raw_w.bitcast(_U32)
            dep = zero
            for g in range(D // 16):
                for i in range(8):
                    ev = ru[jj, pl.ds((16 * g + 2 * i) * 8, 8), :] | dep
                    od = ru[jj, pl.ds((16 * g + 2 * i + 1) * 8, 8), :] | dep
                    lo = (ev & _U32(0xFFFF)) | (od << 16)
                    hi = (ev >> 16) | (od & _U32(0xFFFF0000))
                    wqkv[jj, pl.ds(8 * g + i, H // 2, stride=HP), :] = lo
                    wqkv[jj, pl.ds((H // 2) * HP + 8 * g + i, H // 2, stride=HP), :] = hi
                for _ in range(int("1")):
                    dep = pltpu.roll(hi & zero if _ == 0 else dep, 1, 1)

        NU = 2 * DP // 128 - 1

        def fuse_vo(p, _):
            def wv(pos):
                rows = pl.ds(pl.multiple_of(pos * HP, 8), D // 2)
                tiles = [wqkv[2 * (E // 128) + ec, rows, :] for ec in range(E // 128)]
                return pltpu.bitcast(jnp.concatenate(tiles, axis=1), _BF16)
            r0 = pl.multiple_of(2 * p * D, 64)
            pad = jnp.zeros((DP - D, E), _BF16)
            cut = D // 128 * 128
            even = _dot_nt(wv(p), jnp.concatenate([raw_o[pl.ds(r0, D), :], pad], axis=0))
            odd = _dot_nt(wv(H // 2 + p), jnp.concatenate(
                [pad, raw_o[pl.ds(r0 + D + cut, D - cut), :], raw_o[pl.ds(r0 + D, cut), :]], axis=0))
            nt = DP // 128
            tiles = [even[:, 128 * j:128 * (j + 1)] for j in range(nt - 1)]
            tiles.append(even[:, 128 * (nt - 1):] + odd[:, :128])
            tiles += [odd[:, 128 * j:128 * (j + 1)] for j in range(1, nt)]
            for j, t in enumerate(tiles):
                u_s[p * NU + j, pl.ds(0, D // 2), :] = pltpu.bitcast(t.astype(_BF16), _U32)
            return _

        def ffn_up(i, chunks=None, after_load=None):
            xb = xn[pl.ds(_aligned(i * FB, FB), FB), :]
            if after_load is not None:
                after_load()
            for c in chunks if chunks is not None else range(F // CW):
                half = _dot(xb, w1[:, pl.ds(c * CW, CW)]) * 0.5
                act_s[i % 2, :, pl.ds(c * CW, CW)] = (half * jnp.tanh(half) + half).astype(_BF16)

        def ffn_down(i):
            cols = pl.ds(_aligned(i * FB, FB), FB)
            w = D // 2
            for n in range(2):
                rows = pl.ds(n * w, w)
                baset[rows, cols] = _dot_nt(w2t[rows, :], act_s[i % 2]) + xt[rows, cols].astype(_F32)

        def ffn(i):
            LP = "2"
            ln = (lambda: layer_norm(i + 2)) if (not isinstance(i, int) or i + 2 < NB) else (lambda: None)
            if LP == "0":
                ffn_up(i + 1, None, ln)
                ffn_down(i)
            elif LP == "1":
                ffn_up(i + 1)
                ln()
                ffn_down(i)
            elif LP == "2":
                ffn_up(i + 1)
                ffn_down(i)
                ln()
            elif LP == "3":
                ffn_down(i)
                ffn_up(i + 1)
                ln()
            elif LP == "4":
                ffn_down(i)
                ffn_up(i + 1, None, ln)

        with jax.named_scope("first"):
            cp_x0.wait()
            layer_norm(0)
            for n, (c, (a, b)) in enumerate(zip(cp_1, W1P)):
                c.wait()
                if n == len(W1P) - 1:
                    cp_x1.wait()
                ffn_up(0, range(a, b))
            layer_norm(1)
            ffn_up(1)
        with jax.named_scope("w2wait"):
            cp_2.wait()
        with jax.named_scope("x2wait"):
            cp_x2.wait()
        with jax.named_scope("second"):
            ffn_down(0)
            layer_norm(2)
        with jax.named_scope("x3wait"):
            cp_x3.wait()
        with jax.named_scope("loopA"):
            def ffn_a(it, _):
                i = it + 1
                pltpu.make_async_copy(raw_w.at[it], raw_w.at[it], sems.at[4 + it]).wait()
                retile(it, zero_s[...])
                ffn_up(i + 1)
                ffn_down(i)
                layer_norm(jnp.minimum(i + 2, NB - 1))
                return _
            jax.lax.fori_loop(0, NB - 2, ffn_a, 0, unroll=int("1"))
        with jax.named_scope("last"):
            cp_att[-1].wait()
            ffn_down(NB - 1)

        with jax.named_scope("fuse_vo"):
            jax.lax.fori_loop(0, H // 2, fuse_vo, 0, unroll=int("8"))

        cp_m.wait()
        row = jax.lax.broadcasted_iota(jnp.int32, (L, L), 0)
        col = jax.lax.broadcasted_iota(jnp.int32, (L, L), 1)
        mask = (row < M) | (row >= col)
        lane128 = jax.lax.broadcasted_iota(jnp.int32, (L, 128), 1)

        def flush(start, size):
            cols = pl.ds(start, size)
            at = out_s[cols, :].T
            outt_s[pl.ds(0, D), cols] = (baset[pl.ds(0, D), cols] + at[:D].astype(_F32)).astype(_BF16)
            pltpu.make_async_copy(outt_s.at[pl.ds(0, D), cols], outt_hbm.at[:, cols], osem).start()

        def w_qk(h):
            tiles = [wqkv[ct, pl.ds(hpos(h) * HP, DP // 2), :] for ct in range(2 * E // 128)]
            return pltpu.bitcast(jnp.concatenate(tiles, axis=1), _BF16)

        def step(s, mem, ahead, job=None):
            rows = pl.ds(pl.multiple_of(s * SEG, SEG), SEG)
            hl = jnp.concatenate([mem, xn[rows, :]], axis=0)
            qkv, pp, zz, acc = {}, {}, {}, [None]
            NKT = H * L // 128

            def stage_q(h):
                if h in ahead:
                    qkv[h] = jnp.concatenate([_dot(mem, w_qk(h)), ahead[h]], axis=0)
                else:
                    qkv[h] = _dot(hl, w_qk(h))

            def stage_s(h):
                q = qkv[h][:, :E]
                k = qkv[h][:, E:].astype(_BF16)
                sc = jnp.where(mask, _dot_nt(q, k) * scale, -1e9)
                e = jnp.exp(sc - jnp.max(sc, axis=1, keepdims=True))
                p = e / jnp.sum(e, axis=1, keepdims=True)
                p = jnp.concatenate([p, jnp.zeros((L, 128 - L), _F32)], axis=1)
                off = (h * L) % 128
                pp[h] = pltpu.roll(p, off, 1) if off else p

            def stage_z(p):
                nt = NU // 2
                if ("z", p) in ahead:
                    tails = jnp.concatenate([_dot(mem, pltpu.bitcast(u_s[p * NU + nt], _BF16)), ahead["z", p]], axis=0)
                else:
                    tails = _dot(hl, pltpu.bitcast(u_s[p * NU + nt], _BF16))
                odd_tail = pltpu.roll(tails, 64, 1)
                w = jnp.concatenate([u_s[p * NU + j] for j in range(NU) if j != nt], axis=1)
                z = _dot(hl, pltpu.bitcast(w, _BF16))
                zz[2 * p] = jnp.concatenate([z[:, :128 * nt], tails], axis=1)
                zz[2 * p + 1] = jnp.concatenate([z[:, 128 * nt:], odd_tail], axis=1)

            def tile_heads(t):
                return [h for h in range(H) if h * L < (t + 1) * 128 and (h + 1) * L > t * 128]

            def stage_o(t):
                pt = None
                for h in tile_heads(t):
                    lo, hi = max(h * L - t * 128, 0), min((h + 1) * L - t * 128, 128)
                    if hi - lo < L:
                        piece = jnp.where((lane128 >= lo) & (lane128 < hi), pp[h], 0.0)
                    else:
                        piece = pp[h]
                    pt = piece if pt is None else pt + piece
                hs = tile_heads(t)
                zt = jnp.concatenate([zz[h] for h in hs], axis=0)
                r0 = t * 128 - hs[0] * L
                c = _dot(pt, zt[r0:r0 + 128].astype(_BF16))
                acc[0] = c if acc[0] is None else acc[0] + c

            for t in range(H):
                stage_q(t)
                if t >= D1:
                    stage_s(t - D1)
            ns = H - D1
            zord = [(p + Z0) % (H // 2) for p in range(H // 2)]
            for n, p in enumerate(zord):
                stage_z(p)
                if job is not None and n == JP:
                    job(zz[2 * p][:8, :128])
                if ns < H and n >= SZ:
                    stage_s(ns)
                    ns += 1
            while ns < H:
                stage_s(ns)
                ns += 1
            for t in sorted(range(NKT), key=lambda t: max(zord.index(h // 2) for h in tile_heads(t))):
                stage_o(t)
            a = acc[0]
            out_s[rows, :] = a[M:, :].astype(_BF16)

            return a[:M, :]

        m0 = jnp.concatenate([mem0_s[...].astype(_F32), jnp.zeros((M, DP - D), _F32)], axis=1)
        UNR = int("4")
        NAH = int("0")
        OC = int("640")
        n_full = (S - 1) // OC

        SPJ = 128 // (2 * SEG)

        def out_job(blk, pin):
            tb = pl.multiple_of((blk // 2) * 128, 128)
            f0 = pl.multiple_of((blk % 2) * (DP // 2), DP // 2)
            a = pltpu.bitcast(out_s[pl.ds(tb, 128), pl.ds(f0, DP // 2)], _U32)
            if pin is not None:
                zero = pltpu.bitcast(pin, _U32) & zero_s[...]
                a = a | jnp.tile(zero, (a.shape[0] // 8, a.shape[1] // 128))
            res = baset[pl.ds(f0, DP // 2), pl.ds(tb, 128)] + pltpu.bitcast(a, _BF16).T.astype(_F32)
            outt_s[pl.ds(f0, DP // 2), pl.ds(tb, 128)] = res.astype(_BF16)

        def send(tb):
            cols = pl.ds(tb, 128)
            pltpu.make_async_copy(outt_s.at[pl.ds(0, D), cols], outt_hbm.at[:, cols], osem).start()

        JPI = UNR // SPJ

        def steps(it, mem):
            ahead = {}
            for u in range(UNR):
                s = it * UNR + u
                job = None
                if u % SPJ == JU:
                    blk = jnp.maximum(it * JPI + u // SPJ - 2, 0)
                    job = functools.partial(out_job, blk)
                mem = step(s, mem, ahead, job)
                if u + 1 < UNR:
                    xs = xn[pl.ds(pl.multiple_of((s + 1) * SEG, SEG), SEG), :]
                    ahead = {h: _dot(xs, w_qk(h)) for h in range(NAH)}
                    for p in range(int("4")):
                        ahead["z", p] = _dot(xs, pltpu.bitcast(u_s[p * NU + NU // 2], _BF16))

            done = (it + 1) * JPI - 2

            @pl.when(jnp.logical_and(done % 2 == 0, done > 0))
            def _():
                send(pl.multiple_of((done // 2 - 1) * 128, 128))
            return mem

        with jax.named_scope("steps"):
            jax.lax.fori_loop(0, n_seg // UNR, steps, m0)
        with jax.named_scope("final"):
            last = S // 128 - 1
            out_job(2 * last, None)
            out_job(2 * last + 1, None)
            send(last * 128)
            pltpu.make_async_copy(outt_s.at[pl.ds(0, D)], outt_hbm, osem).wait()

    return kernel


@functools.partial(jax.jit, static_argnames=("A_seg_len",))
def pallas_parallel_sum__memory_aug_recurrent_mem_tr__dense_activation_silu__prompt_kernel(
    A_x, A_mem0, A_Wq, A_Wk, A_Wv, A_Wo, A_seg_len, B_x, B_w1, B_w2,
):
    del B_x
    B, S, D = A_x.shape
    M = A_mem0.shape[1]
    _, H, E = A_Wq.shape
    F = B_w1.shape[1]
    SEG = int(A_seg_len)
    DP = -(-D // 128) * 128
    assert B == 1 and S % SEG == 0 and S % 512 == 0
    L = M + SEG
    kernel = _make_kernel(S, D, DP, H, E, M, SEG, F)
    hbm = pl.BlockSpec(memory_space=pltpu.HBM)
    out_t = pl.pallas_call(
        kernel,
        out_shape=pltpu.HBM((D, S), A_x.dtype),
        in_specs=[hbm] * 8,
        out_specs=hbm,
        scratch_shapes=[
            pltpu.VMEM((DP, S), _BF16),
            pltpu.VMEM((M, D), _BF16),
            pltpu.VMEM((3 * (E // 128), D * H, 128), _BF16),
            pltpu.VMEM((H * D, E), _BF16),
            pltpu.VMEM((D, F), _BF16),
            pltpu.VMEM((S, DP), _F32),
            pltpu.VMEM((DP, S), _F32),
            pltpu.VMEM((3 * E // 128, H * (DP // 2 + 8), 128), _U32),
            pltpu.VMEM((H // 2 * (2 * DP // 128 - 1), DP // 2, 128), _U32),
            pltpu.VMEM((DP, F), _BF16),
            pltpu.VMEM((S, DP), _BF16),
            pltpu.VMEM((DP, S), _BF16),
            pltpu.VMEM((2, 256, F), _BF16),
            pltpu.VMEM((8, 128), _U32),
            pltpu.SemaphoreType.DMA((20,)),
            pltpu.SemaphoreType.DMA(()),
        ],
        compiler_params=pltpu.CompilerParams(vmem_limit_bytes=110 * 1024 * 1024),
    )(
        A_x.reshape(S, D).T, A_mem0.reshape(M, D),
        A_Wq.reshape(D * H, E), A_Wk.reshape(D * H, E), A_Wv.reshape(D * H, E),
        A_Wo.transpose(0, 2, 1).reshape(H * D, E), B_w1, B_w2.T,
    )
    return out_t.T.reshape(B, S, D)
```

```python
import functools

import jax
import jax.numpy as jnp
import numpy as np
from jax.experimental import pallas as pl
from jax.experimental.pallas import tpu as pltpu

_F32 = jnp.float32
_BF16 = jnp.bfloat16
_U32 = jnp.uint32


def _dot(a, b):
    return jax.lax.dot_general(a, b, (((1,), (0,)), ((), ())), preferred_element_type=_F32)


def _dot_nt(a, b):
    return jax.lax.dot_general(a, b, (((1,), (1,)), ((), ())), preferred_element_type=_F32)


def _aligned(i, n):
    return i if isinstance(i, int) else pl.multiple_of(i, n)


def _make_kernel(S, D, DP, H, E, M, SEG, F):
    n_seg = S // SEG
    HP = DP // 2 + 8
    hpos = lambda h: (h % 2) * (H // 2) + h // 2
    L = M + SEG
    FB = 256
    CW = 256
    NB = S // FB
    scale = float(E) ** -0.5
    NST = int(n_seg)
    D1, D2 = int("2"), int("6")
    GL = [int(c, 36) for c in "22222222"]
    JP = int("4"); JU = int("1")
    Z0 = int("6"); SZ = int("0")
    PZD = int("-1"); PZK = int("0")

    def kernel(xt_hbm, mem_hbm, wq_hbm, wk_hbm, wv_hbm, wot_hbm, w1_hbm, w2t_hbm, outt_hbm,
               xt, mem0_s, raw_w, raw_o, w2t,
               xn, baset, wqkv, u_s, w1, out_s, outt_s, act_s, zero_s, sems, osem):
        cp_x0 = pltpu.make_async_copy(xt_hbm.at[:, pl.ds(0, FB)], xt.at[pl.ds(0, D), pl.ds(0, FB)], sems.at[0])
        cp_x1 = pltpu.make_async_copy(xt_hbm.at[:, pl.ds(FB, FB)], xt.at[pl.ds(0, D), pl.ds(FB, FB)], sems.at[11])
        cp_x2 = pltpu.make_async_copy(xt_hbm.at[:, pl.ds(2 * FB, FB)], xt.at[pl.ds(0, D), pl.ds(2 * FB, FB)], sems.at[12])
        cp_x3 = pltpu.make_async_copy(xt_hbm.at[:, pl.ds(3 * FB, S - 3 * FB)],
                                      xt.at[pl.ds(0, D), pl.ds(3 * FB, S - 3 * FB)], sems.at[1])
        W1S = [int(c) for c in "0246"] + [F // CW]
        W1P = tuple(zip(W1S[:-1], W1S[1:]))
        cp_1 = [pltpu.make_async_copy(w1_hbm.at[:, pl.ds(a * CW, (b - a) * CW)],
                                      w1.at[pl.ds(0, D), pl.ds(a * CW, (b - a) * CW)], sems.at[13 + n])
                for n, (a, b) in enumerate(W1P)]
        cp_2 = pltpu.make_async_copy(w2t_hbm, w2t, sems.at[2])
        cp_m = pltpu.make_async_copy(mem_hbm, mem0_s, sems.at[3])
        cp_att = []
        for i, src in enumerate((wq_hbm, wk_hbm, wv_hbm)):
            for ec in range(E // 128):
                cp_att.append(pltpu.make_async_copy(
                    src.at[:, pl.ds(ec * 128, 128)], raw_w.at[i * (E // 128) + ec], sems.at[4 + 2 * i + ec]))
        cp_att.append(pltpu.make_async_copy(wot_hbm, raw_o, sems.at[10]))
        for c in [cp_x0] + cp_1[:-1] + [cp_x1, cp_1[-1], cp_2, cp_x2, cp_x3, cp_m] + cp_att:
            c.start()

        xt[pl.ds(D, DP - D), :] = jnp.zeros((DP - D, S), _BF16)
        for h in range(H):
            wqkv[:, pl.ds(h * HP + D // 2, (DP - D) // 2), :] = jnp.zeros((3 * E // 128, (DP - D) // 2, 128), _U32)
        w1[pl.ds(D, DP - D), :] = jnp.zeros((DP - D, F), _BF16)
        u_s[:, pl.ds(D // 2, (DP - D) // 2), :] = jnp.zeros((u_s.shape[0], (DP - D) // 2, 128), _U32)
        zero_s[...] = jnp.zeros((8, 128), _U32)
        baset[pl.ds(D, DP - D), :] = jnp.zeros((DP - D, S), _F32)
        out_s[pl.ds(0, 128), :] = jnp.zeros((128, DP), _BF16)
        lane = jax.lax.broadcasted_iota(jnp.int32, (FB, DP), 1)

        def layer_norm(i):
            r = _aligned(i * FB, FB)
            xf = xt[:, pl.ds(r, FB)].T.astype(_F32)
            mu = jnp.sum(xf, axis=1, keepdims=True) * (1.0 / D)
            c = jnp.where(lane < D, xf - mu, 0.0)
            var = jnp.sum(c * c, axis=1, keepdims=True) * (1.0 / D)
            xn[pl.ds(r, FB), :] = c * jax.lax.rsqrt(var + 1e-5)

        def xpose8(A):
            sub = jax.lax.broadcasted_iota(jnp.int32, A[0].shape, 0)
            A = list(A)
            for k in (4, 2, 1):
                m = (sub & k) != 0
                B = list(A)
                for i in range(8):
                    if i & k == 0:
                        B[i] = jnp.where(m, pltpu.roll(A[i + k], k, 0), A[i])
                        B[i + k] = jnp.where(m, A[i + k], pltpu.roll(A[i], 8 - k, 0))
                A = B
            return A

        def retile(jj, zero):
            ru = raw_w.bitcast(_U32)
            dep = zero
            for g in range(D // 16):
                for i in range(8):
                    ev = ru[jj, pl.ds((16 * g + 2 * i) * 8, 8), :] | dep
                    od = ru[jj, pl.ds((16 * g + 2 * i + 1) * 8, 8), :] | dep
                    lo = (ev & _U32(0xFFFF)) | (od << 16)
                    hi = (ev >> 16) | (od & _U32(0xFFFF0000))
                    wqkv[jj, pl.ds(8 * g + i, H // 2, stride=HP), :] = lo
                    wqkv[jj, pl.ds((H // 2) * HP + 8 * g + i, H // 2, stride=HP), :] = hi
                for _ in range(int("1")):
                    dep = pltpu.roll(hi & zero if _ == 0 else dep, 1, 1)

        NU = 2 * DP // 128 - 1

        def fuse_vo(p, _):
            def wv(pos):
                rows = pl.ds(pl.multiple_of(pos * HP, 8), D // 2)
                tiles = [wqkv[2 * (E // 128) + ec, rows, :] for ec in range(E // 128)]
                return pltpu.bitcast(jnp.concatenate(tiles, axis=1), _BF16)
            r0 = pl.multiple_of(2 * p * D, 64)
            pad = jnp.zeros((DP - D, E), _BF16)
            cut = D // 128 * 128
            even = _dot_nt(wv(p), jnp.concatenate([raw_o[pl.ds(r0, D), :], pad], axis=0))
            odd = _dot_nt(wv(H // 2 + p), jnp.concatenate(
                [pad, raw_o[pl.ds(r0 + D + cut, D - cut), :], raw_o[pl.ds(r0 + D, cut), :]], axis=0))
            nt = DP // 128
            tiles = [even[:, 128 * j:128 * (j + 1)] for j in range(nt - 1)]
            tiles.append(even[:, 128 * (nt - 1):] + odd[:, :128])
            tiles += [odd[:, 128 * j:128 * (j + 1)] for j in range(1, nt)]
            for j, t in enumerate(tiles):
                u_s[p * NU + j, pl.ds(0, D // 2), :] = pltpu.bitcast(t.astype(_BF16), _U32)
            return _

        def ffn_up(i, chunks=None, after_load=None):
            xb = xn[pl.ds(_aligned(i * FB, FB), FB), :]
            if after_load is not None:
                after_load()
            for c in chunks if chunks is not None else range(F // CW):
                half = _dot(xb, w1[:, pl.ds(c * CW, CW)]) * 0.5
                act_s[i % 2, :, pl.ds(c * CW, CW)] = (half * jnp.tanh(half) + half).astype(_BF16)

        def ffn_down(i):
            cols = pl.ds(_aligned(i * FB, FB), FB)
            w = D // 2
            for n in range(2):
                rows = pl.ds(n * w, w)
                baset[rows, cols] = _dot_nt(w2t[rows, :], act_s[i % 2]) + xt[rows, cols].astype(_F32)

        def ffn(i):
            LP = "2"
            ln = (lambda: layer_norm(i + 2)) if (not isinstance(i, int) or i + 2 < NB) else (lambda: None)
            if LP == "0":
                ffn_up(i + 1, None, ln)
                ffn_down(i)
            elif LP == "1":
                ffn_up(i + 1)
                ln()
                ffn_down(i)
            elif LP == "2":
                ffn_up(i + 1)
                ffn_down(i)
                ln()
            elif LP == "3":
                ffn_down(i)
                ffn_up(i + 1)
                ln()
            elif LP == "4":
                ffn_down(i)
                ffn_up(i + 1, None, ln)

        with jax.named_scope("first"):
            cp_x0.wait()
            layer_norm(0)
            for n, (c, (a, b)) in enumerate(zip(cp_1, W1P)):
                c.wait()
                if n == len(W1P) - 1:
                    cp_x1.wait()
                ffn_up(0, range(a, b))
            layer_norm(1)
            ffn_up(1)
        with jax.named_scope("w2wait"):
            cp_2.wait()
        with jax.named_scope("x2wait"):
            cp_x2.wait()
        with jax.named_scope("second"):
            ffn_down(0)
            layer_norm(2)
        with jax.named_scope("x3wait"):
            cp_x3.wait()
        with jax.named_scope("loopA"):
            def ffn_a(it, _):
                i = it + 1
                pltpu.make_async_copy(raw_w.at[it], raw_w.at[it], sems.at[4 + it]).wait()
                if "1" == "1":
                    retile(it, zero_s[...])
                ffn_up(i + 1)
                ffn_down(i)
                if "1" == "1":
                    layer_norm(jnp.minimum(i + 2, NB - 1))
                return _
            jax.lax.fori_loop(0, NB - 2, ffn_a, 0, unroll=int("1"))
        with jax.named_scope("last"):
            cp_att[-1].wait()
            ffn_down(NB - 1)

        with jax.named_scope("fuse_vo"):
            jax.lax.fori_loop(0, H // 2, fuse_vo, 0, unroll=int("8"))

        cp_m.wait()
        row = jax.lax.broadcasted_iota(jnp.int32, (L, L), 0)
        col = jax.lax.broadcasted_iota(jnp.int32, (L, L), 1)
        mask = (row >= SEG) | (col >= SEG) | (row >= col)
        lane128 = jax.lax.broadcasted_iota(jnp.int32, (L, 128), 1)

        def flush(start, size):
            cols = pl.ds(start, size)
            at = out_s[cols, :].T
            outt_s[pl.ds(0, D), cols] = (baset[pl.ds(0, D), cols] + at[:D].astype(_F32)).astype(_BF16)
            pltpu.make_async_copy(outt_s.at[pl.ds(0, D), cols], outt_hbm.at[:, cols], osem).start()

        def w_qk(h):
            tiles = [wqkv[ct, pl.ds(hpos(h) * HP, DP // 2), :] for ct in range(2 * E // 128)]
            return pltpu.bitcast(jnp.concatenate(tiles, axis=1), _BF16)

        def step(s, mem, ahead, job=None):
            rows = pl.ds(pl.multiple_of(s * SEG, SEG), SEG)
            hl = jnp.concatenate([xn[rows, :], mem], axis=0)
            qkv, pp, zz, acc = {}, {}, {}, [None]
            NKT = H * L // 128

            def stage_q(h):
                if h in ahead:
                    qkv[h] = jnp.concatenate([ahead[h], _dot(mem, w_qk(h))], axis=0)
                else:
                    qkv[h] = _dot(hl, w_qk(h))

            def stage_s(h):
                q = qkv[h][:, :E]
                k = qkv[h][:, E:].astype(_BF16)
                sc = jnp.where(mask, _dot_nt(q, k) * scale, -1e9)
                e = jnp.exp(sc - jnp.max(sc, axis=1, keepdims=True))
                p = e / jnp.sum(e, axis=1, keepdims=True)
                p = jnp.concatenate([p, jnp.zeros((L, 128 - L), _F32)], axis=1)
                off = (h * L) % 128
                pp[h] = pltpu.roll(p, off, 1) if off else p

            def stage_z(p):
                nt = NU // 2
                if ("z", p) in ahead:
                    tails = jnp.concatenate([ahead["z", p], _dot(mem, pltpu.bitcast(u_s[p * NU + nt], _BF16))], axis=0)
                else:
                    tails = _dot(hl, pltpu.bitcast(u_s[p * NU + nt], _BF16))
                odd_tail = pltpu.roll(tails, 64, 1)
                w = jnp.concatenate([u_s[p * NU + j] for j in range(NU) if j != nt], axis=1)
                z = _dot(hl, pltpu.bitcast(w, _BF16))
                zz[2 * p] = jnp.concatenate([z[:, :128 * nt], tails], axis=1)
                zz[2 * p + 1] = jnp.concatenate([z[:, 128 * nt:], odd_tail], axis=1)

            def tile_heads(t):
                return [h for h in range(H) if h * L < (t + 1) * 128 and (h + 1) * L > t * 128]

            def stage_o(t):
                pt = None
                for h in tile_heads(t):
                    lo, hi = max(h * L - t * 128, 0), min((h + 1) * L - t * 128, 128)
                    if hi - lo < L:
                        piece = jnp.where((lane128 >= lo) & (lane128 < hi), pp[h], 0.0)
                    else:
                        piece = pp[h]
                    pt = piece if pt is None else pt + piece
                hs = tile_heads(t)
                zt = jnp.concatenate([zz[h] for h in hs], axis=0)
                r0 = t * 128 - hs[0] * L
                pt = jnp.concatenate([pt[SEG:], pt[:SEG]], axis=0)
                c = _dot(pt, zt[r0:r0 + 128].astype(_BF16))
                acc[0] = c if acc[0] is None else acc[0] + c

            for t in range(H):
                stage_q(t)
                if t >= D1:
                    stage_s(t - D1)
            ns = H - D1
            zord = [(p + Z0) % (H // 2) for p in range(H // 2)]
            for n, p in enumerate(zord):
                stage_z(p)
                if job is not None and n == JP:
                    job(zz[2 * p][:8, :128])
                if ns < H and n >= SZ:
                    stage_s(ns)
                    ns += 1
            while ns < H:
                stage_s(ns)
                ns += 1
            for t in sorted(range(NKT), key=lambda t: max(zord.index(h // 2) for h in tile_heads(t))):
                stage_o(t)
            a = acc[0]
            out_s[rows, :] = a[M:, :].astype(_BF16)

            return a[:M, :]

        m0 = jnp.concatenate([mem0_s[...].astype(_F32), jnp.zeros((M, DP - D), _F32)], axis=1)
        UNR = int("4")
        NAH = int("0")
        OC = int("640")
        n_full = (S - 1) // OC

        SPJ = 128 // (2 * SEG)

        def out_job(blk, pin):
            tb = pl.multiple_of((blk // 2) * 128, 128)
            f0 = pl.multiple_of((blk % 2) * (DP // 2), DP // 2)
            a = pltpu.bitcast(out_s[pl.ds(tb, 128), pl.ds(f0, DP // 2)], _U32)
            if pin is not None:
                zero = pltpu.bitcast(pin, _U32) & zero_s[...]
                a = a | jnp.tile(zero, (a.shape[0] // 8, a.shape[1] // 128))
            res = baset[pl.ds(f0, DP // 2), pl.ds(tb, 128)] + pltpu.bitcast(a, _BF16).T.astype(_F32)
            outt_s[pl.ds(f0, DP // 2), pl.ds(tb, 128)] = res.astype(_BF16)

        def send(tb):
            cols = pl.ds(tb, 128)
            pltpu.make_async_copy(outt_s.at[pl.ds(0, D), cols], outt_hbm.at[:, cols], osem).start()

        JPI = UNR // SPJ

        def steps(it, mem):
            ahead = {}
            for u in range(UNR):
                s = it * UNR + u
                job = None
                if u % SPJ == JU:
                    blk = jnp.maximum(it * JPI + u // SPJ - 2, 0)
                    job = functools.partial(out_job, blk)
                mem = step(s, mem, ahead, job)
                if u + 1 < UNR:
                    xs = xn[pl.ds(pl.multiple_of((s + 1) * SEG, SEG), SEG), :]
                    ahead = {h: _dot(xs, w_qk(h)) for h in range(NAH)}
                    for p in range(int("2")):
                        ahead["z", p] = _dot(xs, pltpu.bitcast(u_s[p * NU + NU // 2], _BF16))

            done = (it + 1) * JPI - 2

            @pl.when(jnp.logical_and(done % 2 == 0, done > 0))
            def _():
                send(pl.multiple_of((done // 2 - 1) * 128, 128))
            return mem

        with jax.named_scope("steps"):
            jax.lax.fori_loop(0, n_seg // UNR, steps, m0)
        with jax.named_scope("final"):
            last = S // 128 - 1
            out_job(2 * last, None)
            out_job(2 * last + 1, None)
            send(last * 128)
            pltpu.make_async_copy(outt_s.at[pl.ds(0, D)], outt_hbm, osem).wait()

    return kernel


@functools.partial(jax.jit, static_argnames=("A_seg_len",))
def pallas_parallel_sum__memory_aug_recurrent_mem_tr__dense_activation_silu__prompt_kernel(
    A_x, A_mem0, A_Wq, A_Wk, A_Wv, A_Wo, A_seg_len, B_x, B_w1, B_w2,
):
    del B_x
    B, S, D = A_x.shape
    M = A_mem0.shape[1]
    _, H, E = A_Wq.shape
    F = B_w1.shape[1]
    SEG = int(A_seg_len)
    DP = -(-D // 128) * 128
    assert B == 1 and S % SEG == 0 and S % 512 == 0
    L = M + SEG
    kernel = _make_kernel(S, D, DP, H, E, M, SEG, F)
    hbm = pl.BlockSpec(memory_space=pltpu.HBM)
    out_t = pl.pallas_call(
        kernel,
        out_shape=pltpu.HBM((D, S), A_x.dtype),
        in_specs=[hbm] * 8,
        out_specs=hbm,
        scratch_shapes=[
            pltpu.VMEM((DP, S), _BF16),
            pltpu.VMEM((M, D), _BF16),
            pltpu.VMEM((3 * (E // 128), D * H, 128), _BF16),
            pltpu.VMEM((H * D, E), _BF16),
            pltpu.VMEM((D, F), _BF16),
            pltpu.VMEM((S, DP), _F32),
            pltpu.VMEM((DP, S), _F32),
            pltpu.VMEM((3 * E // 128, H * (DP // 2 + 8), 128), _U32),
            pltpu.VMEM((H // 2 * (2 * DP // 128 - 1), DP // 2, 128), _U32),
            pltpu.VMEM((DP, F), _BF16),
            pltpu.VMEM((S, DP), _BF16),
            pltpu.VMEM((DP, S), _BF16),
            pltpu.VMEM((2, 256, F), _BF16),
            pltpu.VMEM((8, 128), _U32),
            pltpu.SemaphoreType.DMA((20,)),
            pltpu.SemaphoreType.DMA(()),
        ],
        compiler_params=pltpu.CompilerParams(vmem_limit_bytes=110 * 1024 * 1024),
    )(
        A_x.reshape(S, D).T, A_mem0.reshape(M, D),
        A_Wq.reshape(D * H, E), A_Wk.reshape(D * H, E), A_Wv.reshape(D * H, E),
        A_Wo.transpose(0, 2, 1).reshape(H * D, E), B_w1, B_w2.T,
    )
    return out_t.T.reshape(B, S, D)
```

```python
import functools

import jax
import jax.numpy as jnp
from jax.experimental import pallas as pl
from jax.experimental.pallas import tpu as pltpu

_F32 = jnp.float32
_BF16 = jnp.bfloat16
_U32 = jnp.uint32


def _dot(a, b):
    return jax.lax.dot_general(a, b, (((1,), (0,)), ((), ())), preferred_element_type=_F32)


def _dot_nt(a, b):
    return jax.lax.dot_general(a, b, (((1,), (1,)), ((), ())), preferred_element_type=_F32)


def _aligned(i, n):
    return i if isinstance(i, int) else pl.multiple_of(i, n)


def _make_kernel(S, D, DP, H, E, M, SEG, F):
    L = M + SEG
    FB = 256
    CW = 256
    NB = S // FB
    NE = E // 128
    NT = DP // 128
    NU = 2 * NT - 1
    NKT = H * L // 128
    HP = DP // 2 + 8
    UNR = 128 // SEG
    LAG = 2
    AHEAD = 2
    W1P = ((0, 2), (2, 4), (4, 6), (6, F // CW))
    scale = float(E) ** -0.5
    assert DP - D == 64 and NB - 2 == 3 * NE and H * L % 128 == 0 and UNR == 4

    def hpos(h):
        return (h % 2) * (H // 2) + h // 2

    def tile_heads(t):
        return [h for h in range(H) if h * L < (t + 1) * 128 and (h + 1) * L > t * 128]

    def kernel(xt_hbm, mem_hbm, wq_hbm, wk_hbm, wv_hbm, wot_hbm, w1_hbm, w2t_hbm, outt_hbm,
               xt, mem0, raw_w, raw_o, w1, w2t, xn, act, baset, wqkv, u_s, att, outt, zeros,
               sems, osem):
        def x_copy(b0, nb, sem):
            cols = pl.ds(b0 * FB, nb * FB)
            return pltpu.make_async_copy(xt_hbm.at[:, cols], xt.at[pl.ds(0, D), cols], sems.at[sem])

        cp_x = [x_copy(0, 1, 0), x_copy(1, 1, 1), x_copy(2, 1, 2), x_copy(3, NB - 3, 3)]
        cp_w1 = [pltpu.make_async_copy(w1_hbm.at[:, pl.ds(a * CW, (b - a) * CW)],
                                       w1.at[pl.ds(0, D), pl.ds(a * CW, (b - a) * CW)], sems.at[4 + n])
                 for n, (a, b) in enumerate(W1P)]
        cp_w2 = pltpu.make_async_copy(w2t_hbm, w2t, sems.at[8])
        cp_mem = pltpu.make_async_copy(mem_hbm, mem0, sems.at[9])
        cp_wo = pltpu.make_async_copy(wot_hbm, raw_o, sems.at[10])
        QKV_SEM = 11
        cp_qkv = [pltpu.make_async_copy(src.bitcast(_U32).at[:, pl.ds(ec * 128, 128)],
                                        raw_w.at[i * NE + ec], sems.at[QKV_SEM + i * NE + ec])
                  for i, src in enumerate((wq_hbm, wk_hbm, wv_hbm)) for ec in range(NE)]
        for c in ([cp_x[0]] + cp_w1[:-1] + [cp_x[1], cp_w1[-1], cp_w2, cp_x[2], cp_x[3], cp_mem]
                  + cp_qkv + [cp_wo]):
            c.start()

        xt[pl.ds(D, DP - D), :] = jnp.zeros((DP - D, S), _BF16)
        w1[pl.ds(D, DP - D), :] = jnp.zeros((DP - D, F), _BF16)
        for h in range(H):
            wqkv[:, pl.ds(h * HP + D // 2, (DP - D) // 2), :] = jnp.zeros((3 * NE, (DP - D) // 2, 128), _U32)
        u_s[:, pl.ds(D // 2, (DP - D) // 2), :] = jnp.zeros((H // 2 * NU, (DP - D) // 2, 128), _U32)
        baset[pl.ds(D, DP - D), :] = jnp.zeros((DP - D, S), _F32)
        att[pl.ds(0, 128), :] = jnp.zeros((128, DP), _BF16)
        zeros[...] = jnp.zeros((8, 128), _U32)
        lane = jax.lax.broadcasted_iota(jnp.int32, (FB, DP), 1)

        def layer_norm(i):
            tok = pl.ds(_aligned(i * FB, FB), FB)
            xf = xt[:, tok].T.astype(_F32)
            mu = jnp.sum(xf, axis=1, keepdims=True) * (1.0 / D)
            c = jnp.where(lane < D, xf - mu, 0.0)
            var = jnp.sum(c * c, axis=1, keepdims=True) * (1.0 / D)
            xn[tok, :] = c * jax.lax.rsqrt(var + 1e-5)

        def ffn_up(i, chunks=range(F // CW)):
            xb = xn[pl.ds(_aligned(i * FB, FB), FB), :]
            for c in chunks:
                half = _dot(xb, w1[:, pl.ds(c * CW, CW)]) * 0.5
                act[i % 2, :, pl.ds(c * CW, CW)] = (half * jnp.tanh(half) + half).astype(_BF16)

        def ffn_down(i):
            tok = pl.ds(_aligned(i * FB, FB), FB)
            for n in range(2):
                feat = pl.ds(n * (D // 2), D // 2)
                baset[feat, tok] = _dot_nt(w2t[feat, :], act[i % 2]) + xt[feat, tok].astype(_F32)

        def retile(jj):
            zero = zeros[...]
            dep = zero
            for g in range(D // 16):
                for i in range(8):
                    ev = raw_w[jj, pl.ds((16 * g + 2 * i) * (H // 2), H // 2), :] | dep
                    od = raw_w[jj, pl.ds((16 * g + 2 * i + 1) * (H // 2), H // 2), :] | dep
                    even_heads = (ev & _U32(0xFFFF)) | (od << 16)
                    odd_heads = (ev >> 16) | (od & _U32(0xFFFF0000))
                    wqkv[jj, pl.ds(8 * g + i, H // 2, stride=HP), :] = even_heads
                    wqkv[jj, pl.ds((H // 2) * HP + 8 * g + i, H // 2, stride=HP), :] = odd_heads
                dep = pltpu.roll(odd_heads & zero, 1, 1)

        def fuse_vo(p, carry):
            def wv(pos):
                rows = pl.ds(pl.multiple_of(pos * HP, 8), D // 2)
                tiles = [wqkv[2 * NE + ec, rows, :] for ec in range(NE)]
                return pltpu.bitcast(jnp.concatenate(tiles, axis=1), _BF16)
            r0 = pl.multiple_of(2 * p * D, 64)
            cut = D // 128 * 128
            pad = jnp.zeros((DP - D, E), _BF16)
            even = _dot_nt(wv(p), jnp.concatenate([raw_o[pl.ds(r0, D), :], pad], axis=0))
            odd = _dot_nt(wv(H // 2 + p), jnp.concatenate(
                [pad, raw_o[pl.ds(r0 + D + cut, D - cut), :], raw_o[pl.ds(r0 + D, cut), :]], axis=0))
            tiles = [even[:, 128 * j:128 * (j + 1)] for j in range(NT - 1)]
            tiles.append(even[:, 128 * (NT - 1):] + odd[:, :128])
            tiles += [odd[:, 128 * j:128 * (j + 1)] for j in range(1, NT)]
            for j, t in enumerate(tiles):
                u_s[p * NU + j, pl.ds(0, D // 2), :] = pltpu.bitcast(t.astype(_BF16), _U32)
            return carry

        cp_x[0].wait()
        layer_norm(0)
        for n, (a, b) in enumerate(W1P):
            cp_w1[n].wait()
            if n == len(W1P) - 1:
                cp_x[1].wait()
            ffn_up(0, range(a, b))
        layer_norm(1)
        ffn_up(1)
        cp_w2.wait()
        cp_x[2].wait()
        ffn_down(0)
        layer_norm(2)
        cp_x[3].wait()

        def ffn_block(it, carry):
            pltpu.make_async_copy(raw_w.at[it], raw_w.at[it], sems.at[QKV_SEM + it]).wait()
            retile(it)
            ffn_up(it + 2)
            ffn_down(it + 1)
            layer_norm(jnp.minimum(it + 3, NB - 1))
            return carry
        jax.lax.fori_loop(0, NB - 2, ffn_block, 0)
        cp_wo.wait()
        ffn_down(NB - 1)
        jax.lax.fori_loop(0, H // 2, fuse_vo, 0, unroll=True)

        cp_mem.wait()
        row = jax.lax.broadcasted_iota(jnp.int32, (L, L), 0)
        col = jax.lax.broadcasted_iota(jnp.int32, (L, L), 1)
        mask = (row >= SEG) | (col >= SEG) | (row >= col)
        lane128 = jax.lax.broadcasted_iota(jnp.int32, (L, 128), 1)

        def u_tails(p):
            return pltpu.bitcast(u_s[p * NU + NT - 1], _BF16)

        def step(s, mem, ahead, job):
            tok = pl.ds(pl.multiple_of(s * SEG, SEG), SEG)
            hl = jnp.concatenate([xn[tok, :], mem], axis=0)
            qk, prob, val, acc = {}, {}, {}, [None]

            def project(h):
                tiles = [wqkv[ct, pl.ds(hpos(h) * HP, DP // 2), :] for ct in range(2 * NE)]
                qk[h] = _dot(hl, pltpu.bitcast(jnp.concatenate(tiles, axis=1), _BF16))

            def softmax(h):
                sc = _dot_nt(qk[h][:, :E], qk[h][:, E:].astype(_BF16)) * scale
                sc = jnp.where(mask, sc, -1e9)
                e = jnp.exp(sc - jnp.max(sc, axis=1, keepdims=True))
                p = e / jnp.sum(e, axis=1, keepdims=True)
                p = jnp.concatenate([p, jnp.zeros((L, 128 - L), _F32)], axis=1)
                off = (h * L) % 128
                prob[h] = pltpu.roll(p, off, 1) if off else p

            def values(p):
                if p in ahead:
                    tails = jnp.concatenate([ahead[p], _dot(mem, u_tails(p))], axis=0)
                else:
                    tails = _dot(hl, u_tails(p))
                w = jnp.concatenate([u_s[p * NU + j] for j in range(NU) if j != NT - 1], axis=1)
                z = _dot(hl, pltpu.bitcast(w, _BF16))
                val[2 * p] = jnp.concatenate([z[:, :DP - 128], tails], axis=1)
                val[2 * p + 1] = jnp.concatenate([z[:, DP - 128:], pltpu.roll(tails, 64, 1)], axis=1)

            def mix(t):
                heads, pt = tile_heads(t), None
                for h in heads:
                    lo, hi = max(h * L - t * 128, 0), min((h + 1) * L - t * 128, 128)
                    piece = prob[h]
                    if hi - lo < L:
                        piece = jnp.where((lane128 >= lo) & (lane128 < hi), piece, 0.0)
                    pt = piece if pt is None else pt + piece
                pt = jnp.concatenate([pt[SEG:], pt[:SEG]], axis=0)
                r0 = t * 128 - heads[0] * L
                zt = jnp.concatenate([val[h] for h in heads], axis=0)[r0:r0 + 128]
                c = _dot(pt, zt.astype(_BF16))
                acc[0] = c if acc[0] is None else acc[0] + c

            for h in range(H):
                project(h)
                if h >= LAG:
                    softmax(h - LAG)
            pairs = [(p + 6) % (H // 2) for p in range(H // 2)]
            for n, p in enumerate(pairs):
                values(p)
                if job is not None and n == 4:
                    job(val[2 * p][:8, :128])
                if n < LAG:
                    softmax(H - LAG + n)
            for t in sorted(range(NKT), key=lambda t: max(pairs.index(h // 2) for h in tile_heads(t))):
                mix(t)
            att[tok, :] = acc[0][M:, :].astype(_BF16)
            return acc[0][:M, :]

        def out_job(n, pin):
            tok = pl.ds(pl.multiple_of((n // 2) * 128, 128), 128)
            feat = pl.ds(pl.multiple_of((n % 2) * (DP // 2), DP // 2), DP // 2)
            a = pltpu.bitcast(att[tok, feat], _U32)
            if pin is not None:
                zero = pltpu.bitcast(pin, _U32) & zeros[...]
                a = a | jnp.tile(zero, (a.shape[0] // 8, a.shape[1] // 128))
            outt[feat, tok] = (baset[feat, tok] + pltpu.bitcast(a, _BF16).T.astype(_F32)).astype(_BF16)

        def send(start):
            tok = pl.ds(start, 128)
            pltpu.make_async_copy(outt.at[pl.ds(0, D), tok], outt_hbm.at[:, tok], osem).start()

        def block(it, mem):
            ahead = {}
            for u in range(UNR):
                s = it * UNR + u
                job = functools.partial(out_job, jnp.maximum(2 * it + u // 2 - 2, 0)) if u % 2 else None
                mem = step(s, mem, ahead, job)
                if u + 1 < UNR:
                    xs = xn[pl.ds(pl.multiple_of((s + 1) * SEG, SEG), SEG), :]
                    ahead = {p: _dot(xs, u_tails(p)) for p in range(AHEAD)}

            @pl.when(it > 0)
            def _():
                send(pl.multiple_of((it - 1) * 128, 128))
            return mem

        m0 = jnp.concatenate([mem0[...].astype(_F32), jnp.zeros((M, DP - D), _F32)], axis=1)
        jax.lax.fori_loop(0, S // 128, block, m0)
        out_job(2 * (S // 128) - 2, None)
        out_job(2 * (S // 128) - 1, None)
        send(S - 128)
        pltpu.make_async_copy(outt.at[pl.ds(0, D)], outt_hbm, osem).wait()

    return kernel, dict(HP=HP, NU=NU, NE=NE, FB=FB, n_sems=11 + 3 * NE)


@functools.partial(jax.jit, static_argnames=("A_seg_len",))
def pallas_parallel_sum__memory_aug_recurrent_mem_tr__dense_activation_silu__prompt_kernel(
    A_x, A_mem0, A_Wq, A_Wk, A_Wv, A_Wo, A_seg_len, B_x, B_w1, B_w2,
):
    del B_x
    B, S, D = A_x.shape
    M = A_mem0.shape[1]
    _, H, E = A_Wq.shape
    F = B_w1.shape[1]
    SEG = int(A_seg_len)
    DP = -(-D // 128) * 128
    assert B == 1 and S % 256 == 0
    kernel, c = _make_kernel(S, D, DP, H, E, M, SEG, F)
    hbm = pl.BlockSpec(memory_space=pltpu.HBM)
    out_t = pl.pallas_call(
        kernel,
        out_shape=pltpu.HBM((D, S), A_x.dtype),
        in_specs=[hbm] * 8,
        out_specs=hbm,
        scratch_shapes=[
            pltpu.VMEM((DP, S), _BF16),
            pltpu.VMEM((M, D), _BF16),
            pltpu.VMEM((3 * c["NE"], D * H // 2, 128), _U32),
            pltpu.VMEM((H * D, E), _BF16),
            pltpu.VMEM((DP, F), _BF16),
            pltpu.VMEM((D, F), _BF16),
            pltpu.VMEM((S, DP), _F32),
            pltpu.VMEM((2, c["FB"], F), _BF16),
            pltpu.VMEM((DP, S), _F32),
            pltpu.VMEM((3 * c["NE"], H * c["HP"], 128), _U32),
            pltpu.VMEM((H // 2 * c["NU"], DP // 2, 128), _U32),
            pltpu.VMEM((S, DP), _BF16),
            pltpu.VMEM((DP, S), _BF16),
            pltpu.VMEM((8, 128), _U32),
            pltpu.SemaphoreType.DMA((c["n_sems"],)),
            pltpu.SemaphoreType.DMA(()),
        ],
        compiler_params=pltpu.CompilerParams(vmem_limit_bytes=100 * 1024 * 1024),
    )(
        A_x.reshape(S, D).T, A_mem0.reshape(M, D),
        A_Wq.reshape(D * H, E), A_Wk.reshape(D * H, E), A_Wv.reshape(D * H, E),
        A_Wo.transpose(0, 2, 1).reshape(H * D, E), B_w1, B_w2.T,
    )
    return out_t.T.reshape(B, S, D)
```

```python
import functools

import jax
import jax.numpy as jnp
from jax.experimental import pallas as pl
from jax.experimental.pallas import tpu as pltpu

_F32 = jnp.float32
_BF16 = jnp.bfloat16
_U32 = jnp.uint32


def _dot(a, b):
    return jax.lax.dot_general(a, b, (((1,), (0,)), ((), ())), preferred_element_type=_F32)


def _dot_nt(a, b):
    return jax.lax.dot_general(a, b, (((1,), (1,)), ((), ())), preferred_element_type=_F32)


def _aligned(i, n):
    return i if isinstance(i, int) else pl.multiple_of(i, n)


def _make_kernel(S, D, DP, H, E, M, SEG, F):
    L = M + SEG
    FB = 256
    CW = 256
    NB = S // FB
    NE = E // 128
    NT = DP // 128
    NU = 2 * NT - 1
    NKT = H * L // 128
    HP = DP // 2 + 8
    UNR = 128 // SEG
    LAG = 2
    AHEAD = 2
    W1P = ((0, 2), (2, 4), (4, 6), (6, F // CW))
    scale = float(E) ** -0.5
    assert DP - D == 64 and NB - 2 == 3 * NE and H * L % 128 == 0 and UNR == 4

    def hpos(h):
        return (h % 2) * (H // 2) + h // 2

    def tile_heads(t):
        return [h for h in range(H) if h * L < (t + 1) * 128 and (h + 1) * L > t * 128]

    def kernel(xt_hbm, mem_hbm, wq_hbm, wk_hbm, wv_hbm, wot_hbm, w1_hbm, w2t_hbm, outt_hbm,
               xt, mem0, raw_w, raw_o, w1, w2t, xn, act, baset, wqkv, u_s, att, outt, zeros,
               sems, osem):
        def x_copy(b0, nb, sem):
            cols = pl.ds(b0 * FB, nb * FB)
            return pltpu.make_async_copy(xt_hbm.at[:, cols], xt.at[pl.ds(0, D), cols], sems.at[sem])

        cp_x = [x_copy(0, 1, 0), x_copy(1, 1, 1), x_copy(2, 1, 2), x_copy(3, NB - 3, 3)]
        cp_w1 = [pltpu.make_async_copy(w1_hbm.at[:, pl.ds(a * CW, (b - a) * CW)],
                                       w1.at[pl.ds(0, D), pl.ds(a * CW, (b - a) * CW)], sems.at[4 + n])
                 for n, (a, b) in enumerate(W1P)]
        cp_w2 = pltpu.make_async_copy(w2t_hbm, w2t, sems.at[8])
        cp_mem = pltpu.make_async_copy(mem_hbm, mem0, sems.at[9])
        cp_wo = pltpu.make_async_copy(wot_hbm, raw_o, sems.at[10])
        QKV_SEM = 11
        cp_qkv = [pltpu.make_async_copy(src.bitcast(_U32).at[:, pl.ds(ec * 128, 128)],
                                        raw_w.at[i * NE + ec], sems.at[QKV_SEM + i * NE + ec])
                  for i, src in enumerate((wq_hbm, wk_hbm, wv_hbm)) for ec in range(NE)]
        for c in ([cp_x[0]] + cp_w1[:-1] + [cp_x[1], cp_w1[-1], cp_w2, cp_x[2], cp_x[3], cp_mem]
                  + cp_qkv + [cp_wo]):
            c.start()

        xt[pl.ds(D, DP - D), :] = jnp.zeros((DP - D, S), _BF16)
        w1[pl.ds(D, DP - D), :] = jnp.zeros((DP - D, F), _BF16)
        for h in range(H):
            wqkv[:, pl.ds(h * HP + D // 2, (DP - D) // 2), :] = jnp.zeros((3 * NE, (DP - D) // 2, 128), _U32)
        u_s[:, pl.ds(D // 2, (DP - D) // 2), :] = jnp.zeros((H // 2 * NU, (DP - D) // 2, 128), _U32)
        baset[pl.ds(D, DP - D), :] = jnp.zeros((DP - D, S), _F32)
        att[pl.ds(0, 128), :] = jnp.zeros((128, DP), _BF16)
        zeros[...] = jnp.zeros((8, 128), _U32)
        lane = jax.lax.broadcasted_iota(jnp.int32, (FB, DP), 1)

        def layer_norm(i):
            tok = pl.ds(_aligned(i * FB, FB), FB)
            xf = xt[:, tok].T.astype(_F32)
            mu = jnp.sum(xf, axis=1, keepdims=True) * (1.0 / D)
            c = jnp.where(lane < D, xf - mu, 0.0)
            var = jnp.sum(c * c, axis=1, keepdims=True) * (1.0 / D)
            xn[tok, :] = c * jax.lax.rsqrt(var + 1e-5)

        def ffn_up(i, chunks=range(F // CW)):
            xb = xn[pl.ds(_aligned(i * FB, FB), FB), :]
            for c in chunks:
                half = _dot(xb, w1[:, pl.ds(c * CW, CW)]) * 0.5
                act[i % 2, :, pl.ds(c * CW, CW)] = (half * jnp.tanh(half) + half).astype(_BF16)

        def ffn_down(i):
            tok = pl.ds(_aligned(i * FB, FB), FB)
            for n in range(2):
                feat = pl.ds(n * (D // 2), D // 2)
                baset[feat, tok] = _dot_nt(w2t[feat, :], act[i % 2]) + xt[feat, tok].astype(_F32)

        def retile(jj):
            zero = zeros[...]
            dep = zero
            for g in range(D // 16):
                for i in range(8):
                    ev = raw_w[jj, pl.ds((16 * g + 2 * i) * (H // 2), H // 2), :] | dep
                    od = raw_w[jj, pl.ds((16 * g + 2 * i + 1) * (H // 2), H // 2), :] | dep
                    even_heads = (ev & _U32(0xFFFF)) | (od << 16)
                    odd_heads = (ev >> 16) | (od & _U32(0xFFFF0000))
                    wqkv[jj, pl.ds(8 * g + i, H // 2, stride=HP), :] = even_heads
                    wqkv[jj, pl.ds((H // 2) * HP + 8 * g + i, H // 2, stride=HP), :] = odd_heads
                dep = pltpu.roll(odd_heads & zero, 1, 1)

        def fuse_vo(p, carry):
            def wv(pos, nrows):
                rows = pl.ds(pl.multiple_of(pos * HP, 8), nrows // 2)
                tiles = [wqkv[2 * NE + ec, rows, :] for ec in range(NE)]
                return pltpu.bitcast(jnp.concatenate(tiles, axis=1), _BF16)
            r0 = pl.multiple_of(2 * p * D, 64)
            cut = D // 128 * 128
            tails_t = jnp.concatenate(
                [_dot_nt(raw_o[pl.ds(r0 + cut, D - cut), :], wv(p, DP)),
                 _dot_nt(raw_o[pl.ds(r0 + D + cut, D - cut), :], wv(H // 2 + p, DP))], axis=0)
            even = _dot_nt(wv(p, D), raw_o[pl.ds(r0, cut), :])
            odd = _dot_nt(wv(H // 2 + p, D), raw_o[pl.ds(r0 + D, cut), :])
            tiles = [even[:, 128 * j:128 * (j + 1)] for j in range(NT - 1)]
            tiles.append(tails_t.T[:D])
            tiles += [odd[:, 128 * j:128 * (j + 1)] for j in range(NT - 1)]
            for j, t in enumerate(tiles):
                u_s[p * NU + j, pl.ds(0, D // 2), :] = pltpu.bitcast(t.astype(_BF16), _U32)
            return carry

        cp_x[0].wait()
        layer_norm(0)
        for n, (a, b) in enumerate(W1P):
            cp_w1[n].wait()
            if n == len(W1P) - 1:
                cp_x[1].wait()
            ffn_up(0, range(a, b))
        layer_norm(1)
        ffn_up(1)
        cp_w2.wait()
        cp_x[2].wait()
        ffn_down(0)
        layer_norm(2)
        cp_x[3].wait()

        def ffn_block(it, carry):
            pltpu.make_async_copy(raw_w.at[it], raw_w.at[it], sems.at[QKV_SEM + it]).wait()
            retile(it)
            ffn_up(it + 2)
            ffn_down(it + 1)
            layer_norm(jnp.minimum(it + 3, NB - 1))
            return carry
        jax.lax.fori_loop(0, NB - 2, ffn_block, 0)
        cp_wo.wait()
        ffn_down(NB - 1)
        jax.lax.fori_loop(0, H // 2, fuse_vo, 0, unroll=True)

        cp_mem.wait()
        row = jax.lax.broadcasted_iota(jnp.int32, (L, L), 0)
        col = jax.lax.broadcasted_iota(jnp.int32, (L, L), 1)
        mask = (row >= SEG) | (col >= SEG) | (row >= col)
        lane128 = jax.lax.broadcasted_iota(jnp.int32, (L, 128), 1)

        def u_tails(p):
            return pltpu.bitcast(u_s[p * NU + NT - 1], _BF16)

        def step(s, mem, ahead, job):
            tok = pl.ds(pl.multiple_of(s * SEG, SEG), SEG)
            hl = jnp.concatenate([xn[tok, :], mem], axis=0)
            qk, prob, val, acc = {}, {}, {}, [None]

            def project(h):
                tiles = [wqkv[ct, pl.ds(hpos(h) * HP, DP // 2), :] for ct in range(2 * NE)]
                qk[h] = _dot(hl, pltpu.bitcast(jnp.concatenate(tiles, axis=1), _BF16))

            def softmax(h):
                sc = _dot_nt(qk[h][:, :E], qk[h][:, E:].astype(_BF16)) * scale
                sc = jnp.where(mask, sc, -1e9)
                e = jnp.exp(sc - jnp.max(sc, axis=1, keepdims=True))
                p = e / jnp.sum(e, axis=1, keepdims=True)
                p = jnp.concatenate([p, jnp.zeros((L, 128 - L), _F32)], axis=1)
                off = (h * L) % 128
                prob[h] = pltpu.roll(p, off, 1) if off else p

            def values(p):
                if p in ahead:
                    tails = jnp.concatenate([ahead[p], _dot(mem, u_tails(p))], axis=0)
                else:
                    tails = _dot(hl, u_tails(p))
                w = jnp.concatenate([u_s[p * NU + j] for j in range(NU) if j != NT - 1], axis=1)
                z = _dot(hl, pltpu.bitcast(w, _BF16))
                val[2 * p] = jnp.concatenate([z[:, :DP - 128], tails], axis=1)
                val[2 * p + 1] = jnp.concatenate([z[:, DP - 128:], pltpu.roll(tails, 64, 1)], axis=1)

            def mix(t):
                heads, pt = tile_heads(t), None
                for h in heads:
                    lo, hi = max(h * L - t * 128, 0), min((h + 1) * L - t * 128, 128)
                    piece = prob[h]
                    if hi - lo < L:
                        piece = jnp.where((lane128 >= lo) & (lane128 < hi), piece, 0.0)
                    pt = piece if pt is None else pt + piece
                pt = jnp.concatenate([pt[SEG:], pt[:SEG]], axis=0)
                r0 = t * 128 - heads[0] * L
                zt = jnp.concatenate([val[h] for h in heads], axis=0)[r0:r0 + 128]
                c = _dot(pt, zt.astype(_BF16))
                acc[0] = c if acc[0] is None else acc[0] + c

            for h in range(H):
                project(h)
                if h >= LAG:
                    softmax(h - LAG)
            pairs = [(p + 6) % (H // 2) for p in range(H // 2)]
            for n, p in enumerate(pairs):
                values(p)
                if job is not None and n == 4:
                    job(val[2 * p][:8, :128])
                if n < LAG:
                    softmax(H - LAG + n)
            for t in sorted(range(NKT), key=lambda t: max(pairs.index(h // 2) for h in tile_heads(t))):
                mix(t)
            att[tok, :] = acc[0][M:, :].astype(_BF16)
            return acc[0][:M, :]

        def out_job(n, pin):
            tok = pl.ds(pl.multiple_of((n // 2) * 128, 128), 128)
            feat = pl.ds(pl.multiple_of((n % 2) * (DP // 2), DP // 2), DP // 2)
            a = pltpu.bitcast(att[tok, feat], _U32)
            if pin is not None:
                zero = pltpu.bitcast(pin, _U32) & zeros[...]
                a = a | jnp.tile(zero, (a.shape[0] // 8, a.shape[1] // 128))
            outt[feat, tok] = (baset[feat, tok] + pltpu.bitcast(a, _BF16).T.astype(_F32)).astype(_BF16)

        def send(start):
            tok = pl.ds(start, 128)
            pltpu.make_async_copy(outt.at[pl.ds(0, D), tok], outt_hbm.at[:, tok], osem).start()

        def block(it, mem):
            ahead = {}
            for u in range(UNR):
                s = it * UNR + u
                job = functools.partial(out_job, jnp.maximum(2 * it + u // 2 - 2, 0)) if u % 2 else None
                mem = step(s, mem, ahead, job)
                if u + 1 < UNR:
                    xs = xn[pl.ds(pl.multiple_of((s + 1) * SEG, SEG), SEG), :]
                    ahead = {p: _dot(xs, u_tails(p)) for p in range(AHEAD)}

            @pl.when(it > 0)
            def _():
                send(pl.multiple_of((it - 1) * 128, 128))
            return mem

        m0 = jnp.concatenate([mem0[...].astype(_F32), jnp.zeros((M, DP - D), _F32)], axis=1)
        jax.lax.fori_loop(0, S // 128, block, m0)
        out_job(2 * (S // 128) - 2, None)
        out_job(2 * (S // 128) - 1, None)
        send(S - 128)
        pltpu.make_async_copy(outt.at[pl.ds(0, D)], outt_hbm, osem).wait()

    return kernel, dict(HP=HP, NU=NU, NE=NE, FB=FB, n_sems=11 + 3 * NE)


@functools.partial(jax.jit, static_argnames=("A_seg_len",))
def pallas_parallel_sum__memory_aug_recurrent_mem_tr__dense_activation_silu__prompt_kernel(
    A_x, A_mem0, A_Wq, A_Wk, A_Wv, A_Wo, A_seg_len, B_x, B_w1, B_w2,
):
    del B_x
    B, S, D = A_x.shape
    M = A_mem0.shape[1]
    _, H, E = A_Wq.shape
    F = B_w1.shape[1]
    SEG = int(A_seg_len)
    DP = -(-D // 128) * 128
    assert B == 1 and S % 256 == 0
    kernel, c = _make_kernel(S, D, DP, H, E, M, SEG, F)
    hbm = pl.BlockSpec(memory_space=pltpu.HBM)
    out_t = pl.pallas_call(
        kernel,
        out_shape=pltpu.HBM((D, S), A_x.dtype),
        in_specs=[hbm] * 8,
        out_specs=hbm,
        scratch_shapes=[
            pltpu.VMEM((DP, S), _BF16),
            pltpu.VMEM((M, D), _BF16),
            pltpu.VMEM((3 * c["NE"], D * H // 2, 128), _U32),
            pltpu.VMEM((H * D, E), _BF16),
            pltpu.VMEM((DP, F), _BF16),
            pltpu.VMEM((D, F), _BF16),
            pltpu.VMEM((S, DP), _F32),
            pltpu.VMEM((2, c["FB"], F), _BF16),
            pltpu.VMEM((DP, S), _F32),
            pltpu.VMEM((3 * c["NE"], H * c["HP"] + DP // 2 + 32, 128), _U32),
            pltpu.VMEM((H // 2 * c["NU"], DP // 2, 128), _U32),
            pltpu.VMEM((S, DP), _BF16),
            pltpu.VMEM((DP, S), _BF16),
            pltpu.VMEM((8, 128), _U32),
            pltpu.SemaphoreType.DMA((c["n_sems"],)),
            pltpu.SemaphoreType.DMA(()),
        ],
        compiler_params=pltpu.CompilerParams(vmem_limit_bytes=100 * 1024 * 1024),
    )(
        A_x.reshape(S, D).T, A_mem0.reshape(M, D),
        A_Wq.reshape(D * H, E), A_Wk.reshape(D * H, E), A_Wv.reshape(D * H, E),
        A_Wo.transpose(0, 2, 1).reshape(H * D, E), B_w1, B_w2.T,
    )
    return out_t.T.reshape(B, S, D)
```
